```python
import os as _os
_os.environ.setdefault("JAX_PLATFORMS", "cpu")
import jax
import jax.numpy as jnp

def _softmax(x, axis=-1):
    return jax.nn.softmax(x, axis=axis)
def _gelu(x):
    return jax.nn.gelu(x, approximate=True)
def _silu(x):
    return jax.nn.silu(x)
def _sigmoid(x):
    return jax.nn.sigmoid(x)
def _layernorm(x, axis=-1, eps=1e-5):
    m = jnp.mean(x, axis=axis, keepdims=True)
    v = jnp.var(x, axis=axis, keepdims=True)
    return (x - m) / jnp.sqrt(v + eps)
def _scatter_add(tgt, idx, src, axis=0):
    return tgt.at[idx].add(src)
def _segment_sum(src, seg, n):
    return jax.ops.segment_sum(src, seg, n)
class _Rng:
    def __init__(self, key):
        self._k = key
    def _next(self):
        self._k, sub = jax.random.split(self._k)
        return sub
    def normal(self, shape):
        return jax.random.normal(self._next(), shape, dtype=jnp.bfloat16)
    def randint(self, lo, hi, shape):
        return jax.random.randint(self._next(), shape, lo, hi, dtype=jnp.int32)
    def uniform(self, shape, lo=0.0, hi=1.0):
        return jax.random.uniform(self._next(), shape, jnp.bfloat16, lo, hi)
    def permutation(self, n):
        return jax.random.permutation(self._next(), n)


kernel_name = 'interleave_layers__gqa_block_cached__dense_activation_silu__decode'

def setup_inputs():
    _rng = _Rng(jax.random.key(int.from_bytes(__import__("os").urandom(4), "little")))
    _w = (lambda a: (lambda t: t.astype(jnp.bfloat16) if jnp.issubdtype(t.dtype, jnp.floating) else t)(jnp.asarray(a)))
    def _A_setup():
        B, Sq, D = 2, 1, 512
        Hq, Hkv, Sk, Dh = 32, 8, 8192, 128
        assert Hq % Hkv == 0, (Hq, Hkv)
        return {
            "x": _w((lambda *s: _rng.normal(s) * 0.1)(B, Sq, D)),
            "k_cache": _w((lambda *s: _rng.normal(s) * 0.8)(B, Hkv, Sk, Dh)),
            "v_cache": _w((lambda *s: _rng.normal(s) * 1.6)(B, Hkv, Sk, Dh)),
            "wq": _w((lambda *s: _rng.normal(s) * 0.8)(D, Hq * Dh) * (D ** -0.5)),
            "wo": _w((lambda *s: _rng.normal(s) * 1.6)(Hq * Dh, D) * ((Hq * Dh) ** -0.5)),
        }
    _A_in = _A_setup()

    def _B_setup():
        B, S, D, F = 2, 1, 512, 1792
        return {
            "x": _w((lambda *s: _rng.normal(s) * 0.1)(B, S, D)),
            "w1": _w((lambda *s: _rng.normal(s) * 0.4)(D, F) * (D ** -0.5)),
            "w2": _w((lambda *s: _rng.normal(s) * 0.4)(F, D) * (F ** -0.5)),
        }
    _B_in = _B_setup()

    return {
        "A_x": _A_in["x"],
        "A_k_cache": _A_in["k_cache"],
        "A_v_cache": _A_in["v_cache"],
        "A_wq": _A_in["wq"],
        "A_wo": _A_in["wo"],
        "B_x": _B_in["x"],
        "B_w1": _B_in["w1"],
        "B_w2": _B_in["w2"],
    }

def reference(A_x, A_k_cache, A_v_cache, A_wq, A_wo, B_x, B_w1, B_w2):
    def _A_ref(x, k_cache, v_cache, wq, wo):
        B, Sq, D = x.shape
        Hq, Dh = 32, 128
        Hkv = k_cache.shape[1]
        rep = Hq // Hkv
        q = (lambda x, *d: x.transpose(*d))((x @ wq).reshape(B, Sq, Hq, Dh), 0, 2, 1, 3)
        k = jnp.repeat(k_cache, rep, axis=1)
        v = jnp.repeat(v_cache, rep, axis=1)
        scores = jnp.einsum("bhqd,bhkd->bhqk", q, k) * (Dh ** -0.5)
        p = _softmax(scores, axis=-1)
        o = jnp.einsum("bhqk,bhkd->bhqd", p, v)
        return (lambda x, *d: x.transpose(*d))(o, 0, 2, 1, 3).reshape(B, Sq, Hq * Dh) @ wo

    def _B_ref(x, w1, w2):
        h = jnp.einsum("bsd,df->bsf", x, w1)
        h = _silu(h)
        out = jnp.einsum("bsf,fd->bsd", h, w2)
        return out

    x = A_x
    x = x + _A_ref(_layernorm(x, axis=-1), A_k_cache, A_v_cache, A_wq, A_wo)
    x = x + _B_ref(_layernorm(x, axis=-1), B_w1, B_w2)
    x = x + _A_ref(_layernorm(x, axis=-1), A_k_cache, A_v_cache, A_wq, A_wo)
    x = x + _B_ref(_layernorm(x, axis=-1), B_w1, B_w2)
    return x
```

```python
import jax
import jax.numpy as jnp
from jax import lax
import jax.experimental.pallas as pl
import jax.experimental.pallas.tpu as pltpu

_BF16 = jnp.bfloat16
_F32 = jnp.float32
_NT = (((1,), (1,)), ((), ()))
_LN_EPS = 1e-5
_ROWS = 8

_TAIL_SPLITS = (4096, 2048, 1024, 512, 512)


def _kernel_body(dims, x_hbm, k_hbm, v_hbm, wq_hbm, wo_hbm, w1_hbm, w2_hbm,
                 o_ref,
                 x_v, k_v, v_v, kt_v, wq_v, wo_v, w1_v, w2_v,
                 q_v, p_v, linv_v, o_v,
                 sem_w, sem_k, sem_v, sem_t):
    B, D, HKV, SK, DH, REP = dims
    G = REP * DH
    scale = DH ** -0.5

    def w_copy(i):
        src, dst = ((x_hbm, x_v), (wq_hbm, wq_v), (wo_hbm, wo_v),
                    (w1_hbm, w1_v), (w2_hbm, w2_v))[i]
        return pltpu.make_async_copy(src, dst, sem_w.at[i])

    def k_copy(b, h):
        return pltpu.make_async_copy(k_hbm.at[b, h], k_v.at[b, h],
                                     sem_k.at[b * HKV + h])

    def v_copy(b, h):
        return pltpu.make_async_copy(v_hbm.at[b, h], v_v.at[b, h],
                                     sem_v.at[b * HKV + h])

    tail_offs = []
    off = 0
    for n in _TAIL_SPLITS:
        tail_offs.append((off, n))
        off += n
    assert off == SK

    def vt_copy(i):
        o, n = tail_offs[i]
        return pltpu.make_async_copy(
            v_hbm.at[1, HKV - 1, pl.ds(o, n)],
            v_v.at[1, HKV - 1, pl.ds(o, n)], sem_t.at[i])

    for i in range(5):
        w_copy(i).start()
    for h in range(HKV):
        k_copy(0, h).start()
        v_copy(0, h).start()
    for h in range(HKV):
        k_copy(1, h).start()
    for h in range(HKV - 1):
        v_copy(1, h).start()
    for i in range(len(tail_offs)):
        vt_copy(i).start()

    row = lax.broadcasted_iota(jnp.int32, (_ROWS, DH), 0)
    row_in_grp = row % REP
    row_d = lax.broadcasted_iota(jnp.int32, (_ROWS, D), 0)

    def layernorm(x):
        m = jnp.mean(x, axis=-1, keepdims=True)
        xc = x - m
        var = jnp.mean(xc * xc, axis=-1, keepdims=True)
        return xc * lax.rsqrt(var + _LN_EPS)

    def q_group(res, g_local):
        base = g_local * G
        q = res[:, base:base + DH]
        for j in range(1, REP):
            q = jnp.where(row_in_grp == j,
                          res[:, base + j * DH: base + (j + 1) * DH], q)
        return q.astype(_BF16)

    def softmax_p(s):
        s = s * scale
        m = jnp.max(s, axis=-1, keepdims=True)
        p = jnp.exp(s - m)
        l = jnp.sum(p, axis=-1, keepdims=True)
        return p.astype(_BF16), 1.0 / l

    def block_diag(o):
        parts = [jnp.where(row_in_grp == j, o, 0.0) for j in range(REP)]
        return jnp.concatenate(parts, axis=1).astype(_BF16)

    def sum_rows(acc, lo):
        valid = jnp.logical_and(row_d >= lo, row_d < lo + REP)
        r = jnp.sum(jnp.where(valid, acc, 0.0), axis=0, keepdims=True)
        return jnp.broadcast_to(r, (_ROWS, D))

    def ffn(x):
        xn = layernorm(x).astype(_BF16)
        h = jnp.dot(xn, w1_v[...], preferred_element_type=_F32)
        h = h * jax.nn.sigmoid(h)
        return x + jnp.dot(h.astype(_BF16), w2_v[...],
                           preferred_element_type=_F32)

    def q_all(x):
        xn = layernorm(x).astype(_BF16)
        res = jnp.dot(xn, wq_v[...], preferred_element_type=_F32)
        for g in range(HKV):
            q_v[g] = q_group(res, g)

    def wo_all(lo):
        lhs = jnp.concatenate([block_diag(o_v[g]) for g in range(HKV)], axis=1)
        acc = jnp.dot(lhs, wo_v[...], preferred_element_type=_F32)
        return sum_rows(acc, lo)

    def attn_b0(wait):
        def head(h, carry):
            if wait:
                k_copy(0, h).wait()
            s = lax.dot_general(q_v[h], k_v[0, h], _NT,
                                preferred_element_type=_F32)
            p, linv = softmax_p(s)
            if wait:
                v_copy(0, h).wait()
            o = jnp.dot(p, v_v[0, h], preferred_element_type=_F32)
            o_v[h] = o * linv
            return carry
        lax.fori_loop(0, HKV, head, 0)

    w_copy(0).wait()
    x0 = jnp.broadcast_to(x_v[0].astype(_F32), (_ROWS, D))
    x1 = jnp.broadcast_to(x_v[1].astype(_F32), (_ROWS, D))
    x01 = jnp.where(row_d < REP, x0, x1)
    w_copy(1).wait()
    q_all(x01)

    attn_b0(wait=True)
    q1_b1 = [q_v[g] for g in range(HKV)]
    for g in range(HKV):
        p_v[g, :, 0:DH] = q1_b1[g]
    w_copy(2).wait()
    x0 = x0 + wo_all(0)
    w_copy(3).wait()
    w_copy(4).wait()
    x0 = ffn(x0)
    q_all(x0)
    attn_b0(wait=False)
    x0 = x0 + wo_all(0)
    x0 = ffn(x0)
    o_ref[0] = x0[0:1, :].astype(o_ref.dtype)

    eye = (lax.broadcasted_iota(jnp.int32, (DH, DH), 0)
           == lax.broadcasted_iota(jnp.int32, (DH, DH), 1)).astype(_BF16)

    def qkt_head(h, carry):
        q = p_v[h, :, 0:DH]
        lhs = jnp.concatenate([eye, q, q], axis=0)
        k_copy(1, h).wait()
        r = lax.dot_general(lhs, k_v[1, h], _NT, preferred_element_type=_F32)
        kt_v[h] = r[:DH].astype(_BF16)
        p, linv = softmax_p(r[DH:DH + _ROWS])
        p_v[h] = p
        linv_v[h] = jnp.broadcast_to(linv, (_ROWS, DH))
        return carry
    lax.fori_loop(0, HKV, qkt_head, 0)

    def pv_head(h, acc):
        v_copy(1, h).wait()
        o = jnp.dot(p_v[h], v_v[1, h], preferred_element_type=_F32)
        o = o * linv_v[h]
        w = wo_v[pl.ds(pl.multiple_of(h * G, G), G), :]
        return acc + jnp.dot(block_diag(o), w, preferred_element_type=_F32)
    acc = lax.fori_loop(0, HKV - 1, pv_head, jnp.zeros((_ROWS, D), _F32))

    hl = HKV - 1
    o = None
    for i, (o_, n) in enumerate(tail_offs):
        vt_copy(i).wait()
        part = jnp.dot(p_v[hl, :, o_:o_ + n], v_v[1, hl, o_:o_ + n, :],
                       preferred_element_type=_F32)
        o = part if o is None else o + part
    o = o * linv_v[hl]
    acc = acc + jnp.dot(block_diag(o), wo_v[hl * G:(hl + 1) * G, :],
                        preferred_element_type=_F32)
    x1 = x1 + sum_rows(acc, REP)
    x1 = ffn(x1)

    xn = layernorm(x1).astype(_BF16)
    pend = {}
    acc = None
    for step in range(HKV + 1):
        if step < HKV:
            g = step
            res = jnp.dot(xn, wq_v[:, g * G:(g + 1) * G],
                          preferred_element_type=_F32)
            q = q_group(res, 0)
            s = jnp.dot(q, kt_v[g], preferred_element_type=_F32)
            pend[g] = softmax_p(s)
        if step >= 1:
            g = step - 1
            p, linv = pend.pop(g)
            o = jnp.dot(p, v_v[1, g], preferred_element_type=_F32) * linv
            part = jnp.dot(block_diag(o), wo_v[g * G:(g + 1) * G, :],
                           preferred_element_type=_F32)
            acc = part if acc is None else acc + part
    x1 = x1 + sum_rows(acc, 0)
    x1 = ffn(x1)
    o_ref[1] = x1[0:1, :].astype(o_ref.dtype)


@jax.jit
def pallas_interleave_layers__gqa_block_cached__dense_activation_silu__decode_kernel(
    A_x: jax.Array,
    A_k_cache: jax.Array,
    A_v_cache: jax.Array,
    A_wq: jax.Array,
    A_wo: jax.Array,
    B_x: jax.Array,
    B_w1: jax.Array,
    B_w2: jax.Array,
):
    del B_x
    B, SQ, D = A_x.shape
    _, HKV, SK, DH = A_k_cache.shape
    HQ = A_wq.shape[1] // DH
    REP = HQ // HKV
    F = B_w1.shape[1]
    assert B == 2 and SQ == 1 and 2 * REP == _ROWS
    dims = (B, D, HKV, SK, DH, REP)

    def kernel(*refs):
        _kernel_body(dims, *refs)

    any_spec = pl.BlockSpec(memory_space=pl.ANY)
    return pl.pallas_call(
        kernel,
        out_shape=jax.ShapeDtypeStruct((B, SQ, D), A_x.dtype),
        in_specs=[any_spec] * 7,
        out_specs=pl.BlockSpec(memory_space=pltpu.VMEM),
        scratch_shapes=[
            pltpu.VMEM((B, SQ, D), _BF16),
            pltpu.VMEM((B, HKV, SK, DH), _BF16),
            pltpu.VMEM((B, HKV, SK, DH), _BF16),
            pltpu.VMEM((HKV, DH, SK), _BF16),
            pltpu.VMEM((D, HQ * DH), _BF16),
            pltpu.VMEM((HQ * DH, D), _BF16),
            pltpu.VMEM((D, F), _BF16),
            pltpu.VMEM((F, D), _BF16),
            pltpu.VMEM((HKV, _ROWS, DH), _BF16),
            pltpu.VMEM((HKV, _ROWS, SK), _BF16),
            pltpu.VMEM((HKV, _ROWS, DH), _F32),
            pltpu.VMEM((HKV, _ROWS, DH), _F32),
            pltpu.SemaphoreType.DMA((5,)),
            pltpu.SemaphoreType.DMA((B * HKV,)),
            pltpu.SemaphoreType.DMA((B * HKV,)),
            pltpu.SemaphoreType.DMA((len(_TAIL_SPLITS),)),
        ],
        compiler_params=pltpu.CompilerParams(
            vmem_limit_bytes=110 * 1024 * 1024),
    )(A_x, A_k_cache, A_v_cache, A_wq, A_wo, B_w1, B_w2)
```

```python
import jax
import jax.numpy as jnp
from jax import lax
import jax.experimental.pallas as pl
import jax.experimental.pallas.tpu as pltpu

_BF16 = jnp.bfloat16
_F32 = jnp.float32
_NT = (((1,), (1,)), ((), ()))
_LN_EPS = 1e-5
_ROWS = 8
_LOG2E = 1.4426950408889634

_TAIL_SPLITS = (6144, 1536, 512)
_N_SEMS = 9 + len(_TAIL_SPLITS)


def _kernel_body(dims, x_hbm, k_hbm, v_hbm, wq_hbm, wo_hbm, w1_hbm, w2_hbm,
                 o_ref,
                 x_v, k_v, v_v, kt_v, wq_v, wo_v, w1_v, w2_v,
                 q1_v, q2_v, p_v, linv_v, o_v, csq_v, cs1_v,
                 sems):
    B, D, HKV, SK, DH, REP = dims
    G = REP * DH
    HALF = SK // 2
    HH = HKV // 2
    HL = HKV - 1
    qscale = (DH ** -0.5) * _LOG2E

    def cp(src, dst, i):
        return pltpu.make_async_copy(src, dst, sems.at[i])

    def kv_cp(hbm, vm, b, h0, h1, i):
        return cp(hbm.at[b, pl.ds(h0, h1 - h0)], vm.at[b, pl.ds(h0, h1 - h0)], i)

    tail_offs = []
    off = 0
    for n in _TAIL_SPLITS:
        tail_offs.append((off, n))
        off += n
    assert off == SK

    c_x = lambda: cp(x_hbm, x_v, 0)
    c_wq = lambda: cp(wq_hbm, wq_v, 0)
    c_wo = lambda: cp(wo_hbm, wo_v, 1)
    c_w1 = lambda: cp(w1_hbm, w1_v, 1)
    c_w2 = lambda: cp(w2_hbm, w2_v, 1)
    c_k0 = lambda: kv_cp(k_hbm, k_v, 0, 0, HKV, 2)
    c_v0a = lambda: kv_cp(v_hbm, v_v, 0, 0, HH, 3)
    c_v0b = lambda: kv_cp(v_hbm, v_v, 0, HH, HKV, 4)
    c_k1a = lambda: kv_cp(k_hbm, k_v, 1, 0, HH, 5)
    c_k1b = lambda: kv_cp(k_hbm, k_v, 1, HH, HKV, 6)
    c_v1a = lambda: kv_cp(v_hbm, v_v, 1, 0, HH, 7)
    c_v1b = lambda: kv_cp(v_hbm, v_v, 1, HH, HL, 8)

    def c_vt(i):
        o, n = tail_offs[i]
        return cp(v_hbm.at[1, HL, pl.ds(o, n)], v_v.at[1, HL, pl.ds(o, n)], 9 + i)

    for c in (c_x, c_wq, c_wo, c_w1, c_w2, c_k0, c_v0a, c_v0b, c_k1a, c_k1b,
              c_v1a, c_v1b):
        c().start()
    for i in range(len(tail_offs)):
        c_vt(i).start()

    row = lax.broadcasted_iota(jnp.int32, (_ROWS, DH), 0)
    row_in_grp = row % REP
    lo_rows = row < REP
    row_d = lax.broadcasted_iota(jnp.int32, (_ROWS, D), 0)

    def dot(a, b):
        return jnp.dot(a, b, preferred_element_type=_F32)

    def ln_stats(x):
        m = jnp.mean(x, axis=-1, keepdims=True)
        xc = x - m
        var = jnp.mean(xc * xc, axis=-1, keepdims=True)
        return m, xc, lax.rsqrt(var + _LN_EPS)

    def layernorm(x):
        _, xc, r = ln_stats(x)
        return xc * r

    def pick_heads(res):
        q = res[:, 0:DH]
        for j in range(1, REP):
            q = jnp.where(row_in_grp == j, res[:, j * DH:(j + 1) * DH], q)
        return q

    def softmax_p(s):
        m = jnp.max(s, axis=-1, keepdims=True)
        p = jnp.exp2(s - m)
        l = jnp.sum(p, axis=-1, keepdims=True)
        return p.astype(_BF16), m, l

    def block_diag(o):
        parts = [jnp.where(row_in_grp == j, o, 0.0) for j in range(REP)]
        return jnp.concatenate(parts, axis=1).astype(_BF16)

    def sum_rows(acc, lo, n):
        if n < _ROWS:
            valid = jnp.logical_and(row_d >= lo, row_d < lo + n)
            acc = jnp.where(valid, acc, 0.0)
        r = jnp.sum(acc, axis=0, keepdims=True)
        return jnp.broadcast_to(r, (_ROWS, D))

    def silu(h):
        return h * jax.nn.sigmoid(h)

    def ffn(x):
        xn = layernorm(x).astype(_BF16)
        h = silu(dot(xn, w1_v[...]))
        return x + dot(h.astype(_BF16), w2_v[...])

    def q_all(x, q_ref):
        xn = layernorm(x).astype(_BF16)
        res = dot(xn, wq_v[...])
        for g in range(HKV):
            q_ref[g] = (pick_heads(res[:, g * G:(g + 1) * G]) * qscale).astype(_BF16)

    def wo_all(lo):
        lhs = jnp.concatenate([block_diag(o_v[g]) for g in range(HKV)], axis=1)
        return sum_rows(dot(lhs, wo_v[...]), lo, REP)

    c_x().wait()
    c_wq().wait()
    xin = x_v[...].astype(_F32)
    x0 = jnp.broadcast_to(xin[0:1, :], (_ROWS, D))
    x1 = jnp.broadcast_to(xin[1:2, :], (_ROWS, D))
    x01 = jnp.where(row_d < REP, x0, x1)
    q_all(x01, q1_v)
    ones = jnp.ones((_ROWS, D), _BF16)
    csq = dot(ones, wq_v[...])
    for g in range(HKV):
        csq_v[g] = pick_heads(csq[:, g * G:(g + 1) * G])
    c_wo().wait()
    c_w1().wait()
    c_w2().wait()
    cs1_v[...] = dot(ones, w1_v[...])

    c_k0().wait()

    def qk0_head(h, carry):
        s = lax.dot_general(q1_v[h], k_v[0, h], _NT, preferred_element_type=_F32)
        p, _, l = softmax_p(s)
        p_v[h] = p
        linv_v[h] = jnp.broadcast_to(1.0 / l, (_ROWS, DH))
        return carry
    lax.fori_loop(0, HKV, qk0_head, 0)

    def pv0_head(h, carry):
        @pl.when(h == 0)
        def _():
            c_v0a().wait()

        @pl.when(h == HH)
        def _():
            c_v0b().wait()
        o_v[h] = dot(p_v[h], v_v[0, h]) * linv_v[h]
        return carry
    lax.fori_loop(0, HKV, pv0_head, 0)

    x0 = x0 + wo_all(0)
    x0 = ffn(x0)
    q_all(x0, q2_v)

    def attn0_head(h, carry):
        s = lax.dot_general(q2_v[h], k_v[0, h], _NT, preferred_element_type=_F32)
        p, _, l = softmax_p(s)
        o_v[h] = dot(p, v_v[0, h]) * (1.0 / l)
        return carry
    lax.fori_loop(0, HKV, attn0_head, 0)
    x0 = x0 + wo_all(0)
    x0 = ffn(x0)

    eye = (lax.broadcasted_iota(jnp.int32, (DH, DH), 0)
           == lax.broadcasted_iota(jnp.int32, (DH, DH), 1)).astype(_BF16)

    def qkt_head(h, carry):
        @pl.when(h == 0)
        def _():
            c_k1a().wait()

        @pl.when(h == HH)
        def _():
            c_k1b().wait()
        q = q1_v[h]
        lhs = jnp.concatenate([eye, q, q], axis=0)
        r = lax.dot_general(lhs, k_v[1, h], _NT, preferred_element_type=_F32)
        kt_v[h, 0:DH, :] = r[:DH, :HALF].astype(_BF16)
        kt_v[h, DH:2 * DH, :] = r[:DH, HALF:].astype(_BF16)
        p, _, l = softmax_p(r[DH:DH + _ROWS])
        p_v[h] = p
        linv_v[h] = jnp.broadcast_to(1.0 / l, (_ROWS, DH))
        return carry
    lax.fori_loop(0, HKV, qkt_head, 0)

    def pv1_head(h, acc):
        @pl.when(h == 0)
        def _():
            c_v1a().wait()

        @pl.when(h == HH)
        def _():
            c_v1b().wait()
        o = dot(p_v[h], v_v[1, h]) * linv_v[h]
        w = wo_v[pl.ds(pl.multiple_of(h * G, G), G), :]
        return acc + dot(block_diag(o), w)
    acc = lax.fori_loop(0, HL, pv1_head, jnp.zeros((_ROWS, D), _F32))

    _, x1c, _ = ln_stats(x1)
    upd = sum_rows(acc, REP, REP)
    y_part = x1c + upd
    x_part = x1 + upd

    def ffn_tail(x, y):
        yb = y.astype(_BF16)
        m, yc, r = ln_stats(yb.astype(_F32))
        h = (dot(yb, w1_v[...]) - m * cs1_v[...]) * r
        upd = dot(silu(h).astype(_BF16), w2_v[...])
        return x + upd, yc + upd

    for i, (o_, n) in enumerate(tail_offs):
        c_vt(i).wait()
        o = dot(p_v[HL, :, o_:o_ + n], v_v[1, HL, o_:o_ + n, :])
        if i > 0:
            o = o + o_v[HL]
        if i + 1 < len(tail_offs):
            o_v[HL] = o
    o = o * linv_v[HL]
    upd = sum_rows(dot(block_diag(o), wo_v[HL * G:(HL + 1) * G, :]), REP, REP)
    x1, y = ffn_tail(x_part + upd, y_part + upd)

    yb = y.astype(_BF16)
    m, yc, r = ln_stats(yb.astype(_F32))
    rq = r * qscale
    qs = []
    for g in range(HKV):
        res = pick_heads(dot(yb, wq_v[:, g * G:(g + 1) * G]))
        q = (res - m * csq_v[g]) * rq
        qs.append(jnp.concatenate(
            [jnp.where(lo_rows, q, 0.0), jnp.where(lo_rows, 0.0, q)],
            axis=1).astype(_BF16))

    def qk(g):
        p, mx, l = softmax_p(dot(qs[g], kt_v[g]))
        mx = jnp.broadcast_to(mx, (_ROWS, DH))
        l = jnp.broadcast_to(l, (_ROWS, DH))
        mx_all = jnp.maximum(mx, pltpu.roll(mx, REP, axis=0))
        a = jnp.exp2(mx - mx_all)
        al = a * l
        return p, a / (al + pltpu.roll(al, REP, axis=0))

    def pv(g, p, c):
        o_lo = dot(p, v_v[1, g, 0:HALF, :])
        o_hi = dot(p, v_v[1, g, HALF:SK, :])
        return block_diag(jnp.where(lo_rows, o_lo, o_hi) * c)

    def wo(g, lhs):
        return dot(lhs, wo_v[g * G:(g + 1) * G, :])

    ps, os_, acc = {}, {}, None
    for step in range(HKV + 2):
        if step < HKV:
            ps[step] = qk(step)
        if 1 <= step <= HKV:
            os_[step - 1] = pv(step - 1, *ps.pop(step - 1))
        if step >= 2:
            part = wo(step - 2, os_.pop(step - 2))
            acc = part if acc is None else acc + part
    upd = sum_rows(acc, 0, _ROWS)
    x1, _ = ffn_tail(x1 + upd, yc + upd)
    out = jnp.where(row_d < 1, x0, x1)
    o_ref[...] = out[0:B, :].astype(o_ref.dtype)


@jax.jit
def pallas_interleave_layers__gqa_block_cached__dense_activation_silu__decode_kernel(
    A_x: jax.Array,
    A_k_cache: jax.Array,
    A_v_cache: jax.Array,
    A_wq: jax.Array,
    A_wo: jax.Array,
    B_x: jax.Array,
    B_w1: jax.Array,
    B_w2: jax.Array,
):
    del B_x
    B, SQ, D = A_x.shape
    _, HKV, SK, DH = A_k_cache.shape
    HQ = A_wq.shape[1] // DH
    REP = HQ // HKV
    F = B_w1.shape[1]
    assert B == 2 and SQ == 1 and 2 * REP == _ROWS
    dims = (B, D, HKV, SK, DH, REP)

    def kernel(*refs):
        _kernel_body(dims, *refs)

    any_spec = pl.BlockSpec(memory_space=pl.ANY)
    out = pl.pallas_call(
        kernel,
        out_shape=jax.ShapeDtypeStruct((B, D), A_x.dtype),
        in_specs=[any_spec] * 7,
        out_specs=pl.BlockSpec(memory_space=pltpu.VMEM),
        scratch_shapes=[
            pltpu.VMEM((B, D), _BF16),
            pltpu.VMEM((B, HKV, SK, DH), _BF16),
            pltpu.VMEM((B, HKV, SK, DH), _BF16),
            pltpu.VMEM((HKV, 2 * DH, SK // 2), _BF16),
            pltpu.VMEM((D, HQ * DH), _BF16),
            pltpu.VMEM((HQ * DH, D), _BF16),
            pltpu.VMEM((D, F), _BF16),
            pltpu.VMEM((F, D), _BF16),
            pltpu.VMEM((HKV, _ROWS, DH), _BF16),
            pltpu.VMEM((HKV, _ROWS, DH), _BF16),
            pltpu.VMEM((HKV, _ROWS, SK), _BF16),
            pltpu.VMEM((HKV, _ROWS, DH), _F32),
            pltpu.VMEM((HKV, _ROWS, DH), _F32),
            pltpu.VMEM((HKV, _ROWS, DH), _F32),
            pltpu.VMEM((_ROWS, F), _F32),
            pltpu.SemaphoreType.DMA((_N_SEMS,)),
        ],
        compiler_params=pltpu.CompilerParams(
            vmem_limit_bytes=110 * 1024 * 1024),
    )(A_x.reshape(B, D), A_k_cache, A_v_cache, A_wq, A_wo, B_w1, B_w2)
    return out.reshape(B, SQ, D)
```

```python
import jax
import jax.numpy as jnp
from jax import lax
import jax.experimental.pallas as pl
import jax.experimental.pallas.tpu as pltpu

_BF16 = jnp.bfloat16
_F32 = jnp.float32
_U32 = jnp.uint32
_NT = (((1,), (1,)), ((), ()))
_LN_EPS = 1e-5
_ROWS = 8
_LOG2E = 1.4426950408889634

_TAIL_SPLITS = (6144, 1536, 512)
_N_SEMS = 9 + len(_TAIL_SPLITS)
_FV = 640
_N_COLS = 8

_SCHED = ("mq0 wq1 wq2 wq3 wq4 wq5 wq6 wq7 qa0 qb0 qa1 qb1 pl0 ph0 qa2 qb2 "
          "pl1 ph1 qa3 wo0 tk qb3 pl2 ph2 qa4 wo1 tk qb4 pl3 ph3 qa5 wo2 tk "
          "qb5 pl4 ph4 qa6 wo3 tk qb6 pl5 ph5 qa7 wo4 tk qb7 pl6 ph6 wo5 tk "
          "pl7 ph7 wo6 mo7")


def _kernel_body(dims, x_hbm, k_hbm, v_hbm, wq_hbm, wo_hbm, w1_hbm, w2_hbm,
                 o_ref,
                 x_v, k_v, v_v, kt_v, wq_v, wo_v, w1_v, w2_v,
                 q1_v, q2_v, p_v, linv_v, o_v, csq_v, cs1_v,
                 wqp_v, wop_v, w1p_v, w2p_v, w1t_v, cs1c_v, w2f_v,
                 *rest):
    col_v, sems = rest[:_N_COLS], rest[_N_COLS]
    B, D, HKV, SK, DH, REP, F = dims
    G = REP * DH
    HALF = SK // 2
    HH = HKV // 2
    HL = HKV - 1
    FM = F - _FV
    qscale = (DH ** -0.5) * _LOG2E

    def cp(src, dst, i):
        return pltpu.make_async_copy(src, dst, sems.at[i])

    def kv_cp(hbm, vm, b, h0, h1, i):
        return cp(hbm.at[b, pl.ds(h0, h1 - h0)], vm.at[b, pl.ds(h0, h1 - h0)], i)

    tail_offs = []
    off = 0
    for n in _TAIL_SPLITS:
        tail_offs.append((off, n))
        off += n
    assert off == SK

    c_x = lambda: cp(x_hbm, x_v, 0)
    c_wq = lambda: cp(wq_hbm, wq_v, 0)
    c_wo = lambda: cp(wo_hbm, wo_v, 1)
    c_w1 = lambda: cp(w1_hbm, w1_v, 1)
    c_w2 = lambda: cp(w2_hbm, w2_v, 1)
    c_k0 = lambda: kv_cp(k_hbm, k_v, 0, 0, HKV, 2)
    c_v0a = lambda: kv_cp(v_hbm, v_v, 0, 0, HH, 3)
    c_v0b = lambda: kv_cp(v_hbm, v_v, 0, HH, HKV, 4)
    c_k1a = lambda: kv_cp(k_hbm, k_v, 1, 0, HH, 5)
    c_k1b = lambda: kv_cp(k_hbm, k_v, 1, HH, HKV, 6)
    c_v1a = lambda: kv_cp(v_hbm, v_v, 1, 0, HH, 7)
    c_v1b = lambda: kv_cp(v_hbm, v_v, 1, HH, HL, 8)

    def c_vt(i):
        o, n = tail_offs[i]
        return cp(v_hbm.at[1, HL, pl.ds(o, n)], v_v.at[1, HL, pl.ds(o, n)], 9 + i)

    for c in (c_x, c_wq, c_wo, c_w1, c_w2, c_k0, c_v0a, c_v0b, c_k1a, c_k1b,
              c_v1a, c_v1b):
        c().start()
    for i in range(len(tail_offs)):
        c_vt(i).start()

    row = lax.broadcasted_iota(jnp.int32, (_ROWS, DH), 0)
    row_in_grp = row % REP
    lo_rows = row < REP
    row_d = lax.broadcasted_iota(jnp.int32, (_ROWS, D), 0)

    def dot(a, b):
        return jnp.dot(a, b, preferred_element_type=_F32)

    def pack(x):
        return pltpu.bitcast(x, _U32)

    def unpack(x):
        return pltpu.bitcast(x, _BF16)

    vu_v = v_v.bitcast(_U32)

    def ln_stats(x):
        m = jnp.mean(x, axis=-1, keepdims=True)
        xc = x - m
        var = jnp.mean(xc * xc, axis=-1, keepdims=True)
        return m, xc, lax.rsqrt(var + _LN_EPS)

    def ln_stats1(x):
        m = jnp.mean(x, axis=-1, keepdims=True)
        m2 = jnp.mean(x * x, axis=-1, keepdims=True)
        var = jnp.maximum(m2 - m * m, 0.0)
        return m, x - m, lax.rsqrt(var + _LN_EPS)

    def layernorm(x):
        _, xc, r = ln_stats(x)
        return xc * r

    def pick_heads(res):
        q = res[:, 0:DH]
        for j in range(1, REP):
            q = jnp.where(row_in_grp == j, res[:, j * DH:(j + 1) * DH], q)
        return q

    def softmax_p(s):
        m = jnp.max(s, axis=-1, keepdims=True)
        p = jnp.exp2(s - m)
        l = jnp.sum(p, axis=-1, keepdims=True)
        return p.astype(_BF16), m, l

    def block_diag(o):
        parts = [jnp.where(row_in_grp == j, o, 0.0) for j in range(REP)]
        return jnp.concatenate(parts, axis=1).astype(_BF16)

    def sum_rows(acc, lo, n):
        if n < _ROWS:
            valid = jnp.logical_and(row_d >= lo, row_d < lo + n)
            acc = jnp.where(valid, acc, 0.0)
        r = jnp.sum(acc, axis=0, keepdims=True)
        return jnp.broadcast_to(r, (_ROWS, D))

    def silu_half(hh):
        return hh + hh * jnp.tanh(hh)

    def ffn(x):
        xn = layernorm(x).astype(_BF16)
        h = silu_half(0.5 * dot(xn, w1_v[...]))
        return x + dot(h.astype(_BF16), w2_v[...])

    def q_all(x, q_ref):
        xn = layernorm(x).astype(_BF16)
        res = dot(xn, wq_v[...])
        for g in range(HKV):
            q_ref[g] = (pick_heads(res[:, g * G:(g + 1) * G]) * qscale).astype(_BF16)

    def wo_all(lo):
        lhs = jnp.concatenate([block_diag(o_v[g]) for g in range(HKV)], axis=1)
        return sum_rows(dot(lhs, wo_v[...]), lo, REP)

    c_x().wait()
    c_wq().wait()
    xin = x_v[...].astype(_F32)
    x0 = jnp.broadcast_to(xin[0:1, :], (_ROWS, D))
    x1 = jnp.broadcast_to(xin[1:2, :], (_ROWS, D))
    x01 = jnp.where(row_d < REP, x0, x1)
    q_all(x01, q1_v)

    ones = jnp.ones((_ROWS, D), _BF16)
    csq = dot(ones, wq_v[...])
    for g in range(HKV):
        csq_v[g] = pick_heads(csq[:, g * G:(g + 1) * G])
    c_wo().wait()
    c_w1().wait()
    c_w2().wait()
    cs1_v[...] = dot(ones, w1_v[...])
    for src, dst in ((wq_v, wqp_v), (wo_v, wop_v), (w1_v, w1p_v), (w2_v, w2p_v)):
        def pack_rows(i, carry, src=src, dst=dst):
            r0 = pl.multiple_of(i * 64, 64)
            r1 = pl.multiple_of(i * 32, 32)
            dst[pl.ds(r1, 32), :] = pack(src[pl.ds(r0, 64), :])
            return carry
        lax.fori_loop(0, src.shape[0] // 64, pack_rows, 0)
    w1t = w1_v[:, FM:F].astype(_F32).T
    w1t_v[...] = w1t
    w2f_v[...] = w2_v[FM:F, :].astype(_F32)
    cs1c_v[...] = jnp.broadcast_to(jnp.sum(w1t, axis=1, keepdims=True), (_FV, DH))
    for c in col_v:
        c[2 * DH:2 * DH + 8, :] = jnp.zeros((8, DH), _U32)

    c_k0().wait()

    def qk0_head(h, carry):
        s = lax.dot_general(q1_v[h], k_v[0, h], _NT, preferred_element_type=_F32)
        p, _, l = softmax_p(s)
        p_v[h] = p
        linv_v[h] = jnp.broadcast_to(1.0 / l, (_ROWS, DH))
        return carry
    lax.fori_loop(0, HKV, qk0_head, 0)

    def pv0_head(h, carry):
        @pl.when(h == 0)
        def _():
            c_v0a().wait()

        @pl.when(h == HH)
        def _():
            c_v0b().wait()
        o_v[h] = dot(p_v[h], v_v[0, h]) * linv_v[h]
        return carry
    lax.fori_loop(0, HKV, pv0_head, 0)

    x0 = x0 + wo_all(0)
    x0 = ffn(x0)
    q_all(x0, q2_v)

    def attn0_head(h, carry):
        s = lax.dot_general(q2_v[h], k_v[0, h], _NT, preferred_element_type=_F32)
        p, _, l = softmax_p(s)
        o_v[h] = dot(p, v_v[0, h]) * (1.0 / l)
        return carry
    lax.fori_loop(0, HKV, attn0_head, 0)
    x0 = x0 + wo_all(0)
    x0 = ffn(x0)

    eye = (lax.broadcasted_iota(jnp.int32, (DH, DH), 0)
           == lax.broadcasted_iota(jnp.int32, (DH, DH), 1)).astype(_BF16)

    def qkt_head(h, carry):
        @pl.when(h == 0)
        def _():
            c_k1a().wait()

        @pl.when(h == HH)
        def _():
            c_k1b().wait()
        q = q1_v[h]
        lhs = jnp.concatenate([eye, q, q], axis=0)
        r = lax.dot_general(lhs, k_v[1, h], _NT, preferred_element_type=_F32)
        kt_v[h, 0:DH // 2, :] = pack(r[:DH, :HALF].astype(_BF16))
        kt_v[h, DH // 2:DH, :] = pack(r[:DH, HALF:].astype(_BF16))
        p, _, l = softmax_p(r[DH:DH + _ROWS])
        p_v[h] = p
        linv_v[h] = jnp.broadcast_to(1.0 / l, (_ROWS, DH))
        return carry + h
    zero = lax.fori_loop(0, HKV, qkt_head, 0) - (HKV * (HKV - 1)) // 2
    zero = jnp.clip(zero, 0, 1)

    def pv1_head(h, acc):
        @pl.when(h == 0)
        def _():
            c_v1a().wait()

        @pl.when(h == HH)
        def _():
            c_v1b().wait()
        o = dot(p_v[h], v_v[1, h]) * linv_v[h]
        w = wo_v[pl.ds(pl.multiple_of(h * G, G), G), :]
        return acc + dot(block_diag(o), w)
    acc = lax.fori_loop(0, HL, pv1_head, jnp.zeros((_ROWS, D), _F32))

    _, x1c, _ = ln_stats(x1)
    upd = sum_rows(acc, REP, REP)
    y_part = x1c + upd
    x_part = x1 + upd

    def ffn_tail(x, y):
        yb = y.astype(_BF16)
        yf = yb.astype(_F32)
        m, yc, r = ln_stats1(yf)
        rh = 0.5 * r
        hh = (dot(yb, unpack(w1p_v[:, 0:FM])) - m * cs1_v[:, 0:FM]) * rh
        upd = dot(silu_half(hh).astype(_BF16), unpack(w2p_v[0:FM // 2, :]))
        a = None
        for nb in range(_FV // 8):
            t = w1t_v[nb * 8:(nb + 1) * 8, :] * yf
            t = (t[:, 0:DH] + t[:, DH:2 * DH]) + (t[:, 2 * DH:3 * DH] + t[:, 3 * DH:])
            hs = jnp.sum(t, axis=1, keepdims=True)
            hc = silu_half((hs - m * cs1c_v[nb * 8:(nb + 1) * 8, :]) * rh)
            u = w2f_v[nb * 8:(nb + 1) * 8, :] * jnp.concatenate([hc] * (D // DH), axis=1)
            a = u if a is None else a + u
        upd = upd + sum_rows(a, 0, _ROWS)
        return x + upd, yc + upd

    for i, (o_, n) in enumerate(tail_offs):
        c_vt(i).wait()
        o = dot(p_v[HL, :, o_:o_ + n], unpack(vu_v[1, HL, o_ // 2:(o_ + n) // 2, :]))
        if i > 0:
            o = o + o_v[HL]
        if i + 1 < len(tail_offs):
            o_v[HL] = o
    o = o * linv_v[HL]
    upd = sum_rows(dot(block_diag(o), unpack(wop_v[HL * G // 2:(HL + 1) * G // 2, :])),
                   REP, REP)
    x1, y = ffn_tail(x_part + upd, y_part + upd)

    def to_col(rows, col_ref):
        u = [pltpu.bitcast(jnp.broadcast_to(r_, (_ROWS, DH)), _U32) for r_ in rows]
        pk = [(u[0] >> 16) | u[1], (u[2] >> 16) | u[3]]
        rep = jnp.concatenate(
            [jnp.broadcast_to(p_[0:1, :], (DH, DH)) for p_ in pk], axis=1)
        col_ref[0:2 * DH, :] = rep.T

    def col_pair(col_ref, i):
        u = col_ref[pl.ds(pl.multiple_of((zero + i) * 8, 8), 8), :]
        return (pltpu.bitcast(u << 16, _F32),
                pltpu.bitcast(u & jnp.uint32(0xFFFF0000), _F32))

    toks = []

    def gate(x):
        while toks:
            x = jnp.where(zero != 0, toks.pop().astype(x.dtype), x)
        return x

    last = [None] * 4

    def vpu_matvec(col_ref, wp_ref, r0, c0):
        accs = [None] * 4
        for p_ in range(2):
            for kb in range(DH // 16):
                cks = [col_pair(col_ref, p_ * (DH // 8) + kb * 2 + sub)
                       for sub in range(2)]
                for hl in range(2):
                    rr = (r0 + (2 * p_ + hl) * DH) // 2 + kb * 8
                    ws = [unpack(wp_ref[rr:rr + 8, c0 + j * DH:c0 + (j + 1) * DH]
                                 ).astype(_F32) for j in range(4)]
                    for sub in range(2):
                        for j in range(4):
                            t = ws[j][sub * 8:(sub + 1) * 8, :] * cks[sub][hl]
                            accs[j] = t if accs[j] is None else accs[j] + t
        last[:] = accs
        return accs

    def fold_rows(a):
        def fold(x, y_, sh):
            msk = (row % (2 * sh)) < sh
            if 2 * sh == _ROWS:
                return (jnp.where(msk, x, y_)
                        + pltpu.roll(jnp.where(msk, y_, x), sh, axis=0))
            return jnp.where(msk, x + pltpu.roll(x, _ROWS - sh, axis=0),
                             y_ + pltpu.roll(y_, sh, axis=0))
        b = [fold(a[i], a[i + 4], 4) for i in range(4)]
        c = [fold(b[i], b[i + 2], 2) for i in range(2)]
        return fold(c[0], c[1], 1)

    yb = y.astype(_BF16)
    yf = yb.astype(_F32)
    m, yc, r = ln_stats1(yf)
    rq = r * qscale
    to_col([yf[0:1, j * DH:(j + 1) * DH] for j in range(D // DH)], col_v[0])
    qb, sm, ps, oh, os_ = {}, {}, {}, {}, {}
    st = {"mx": None, "vp": None}

    def finish_q(g, res):
        qb[g] = ((res - m * csq_v[g]) * rq).astype(_BF16)

    def t_mq(g):
        finish_q(g, pick_heads(dot(yb, unpack(wqp_v[:, g * G:(g + 1) * G]))))

    def t_wq(g):
        accs = vpu_matvec(col_v[0], wqp_v, 0, g * G)
        finish_q(g, fold_rows(accs + accs))

    def t_tk():
        toks.append((last[0] + last[1]) + (last[2] + last[3]))

    def t_q(g, part):
        q = gate(qb[g])
        zq = jnp.zeros_like(q)
        q2 = jnp.concatenate(
            [jnp.where(lo_rows, q, zq), jnp.where(lo_rows, zq, q)], axis=1)
        c0 = part * (HALF // 2)
        sm.setdefault(g, []).append(dot(q2, unpack(kt_v[g, :, c0:c0 + HALF // 2])))

    def t_sm(g):
        p, mx, l = softmax_p(jnp.concatenate(sm.pop(g), axis=1))
        mx = jnp.broadcast_to(mx, (_ROWS, DH))
        l = jnp.broadcast_to(l, (_ROWS, DH))
        mx_all = jnp.maximum(mx, pltpu.roll(mx, REP, axis=0))
        a = jnp.exp2(mx - mx_all)
        al = a * l
        ps[g] = (p, a / (al + pltpu.roll(al, REP, axis=0)))

    def t_p(g, part):
        if g not in ps:
            t_sm(g)
        p, c = ps[g]
        if toks:
            tk = list(toks)
            pieces = []
            for i in range(4):
                toks[:] = tk
                pieces.append(gate(p[:, i * DH:(i + 1) * DH]))
            p = jnp.concatenate(pieces + [p[:, 4 * DH:]], axis=1)
        o = dot(p, unpack(vu_v[1, g, part * (HALF // 2):(part + 1) * (HALF // 2), :]))
        if part == 0:
            oh[g] = o
        else:
            os_[g] = jnp.where(lo_rows, oh.pop(g), o) * c

    def t_mo(g):
        part = dot(block_diag(gate(os_.pop(g))),
                   unpack(wop_v[g * G // 2:(g + 1) * G // 2, :]))
        st["mx"] = part if st["mx"] is None else part + st["mx"]

    def t_wo(g):
        o = os_.pop(g)
        o4 = (o + pltpu.roll(o, REP, axis=0)).astype(_BF16).astype(_F32)
        to_col([o4[j:j + 1, :] for j in range(REP)], col_v[1 + g])
        part = jnp.concatenate(vpu_matvec(col_v[1 + g], wop_v, g * G, 0), axis=1)
        st["vp"] = part if st["vp"] is None else st["vp"] + part

    tasks = {"mq": t_mq, "wq": t_wq, "tk": t_tk, "mo": t_mo, "wo": t_wo,
             "qa": lambda g: t_q(g, 0), "qb": lambda g: t_q(g, 1),
             "pl": lambda g: t_p(g, 0), "ph": lambda g: t_p(g, 1)}
    for item in _SCHED.split():
        tasks[item[:2]](*[int(c) for c in item[2:]])
    assert not os_ and not toks
    upd = sum_rows(st["mx"] + st["vp"], 0, _ROWS)
    x1, _ = ffn_tail(x1 + upd, yc + upd)
    out = jnp.where(row_d < 1, x0, x1)
    o_ref[...] = out[0:B, :].astype(o_ref.dtype)


@jax.jit
def pallas_interleave_layers__gqa_block_cached__dense_activation_silu__decode_kernel(
    A_x: jax.Array,
    A_k_cache: jax.Array,
    A_v_cache: jax.Array,
    A_wq: jax.Array,
    A_wo: jax.Array,
    B_x: jax.Array,
    B_w1: jax.Array,
    B_w2: jax.Array,
):
    del B_x
    B, SQ, D = A_x.shape
    _, HKV, SK, DH = A_k_cache.shape
    HQ = A_wq.shape[1] // DH
    REP = HQ // HKV
    F = B_w1.shape[1]
    assert B == 2 and SQ == 1 and 2 * REP == _ROWS and HKV == 8
    assert D == REP * DH and DH == 128
    dims = (B, D, HKV, SK, DH, REP, F)

    def kernel(*refs):
        _kernel_body(dims, *refs)

    any_spec = pl.BlockSpec(memory_space=pl.ANY)
    out = pl.pallas_call(
        kernel,
        out_shape=jax.ShapeDtypeStruct((B, D), A_x.dtype),
        in_specs=[any_spec] * 7,
        out_specs=pl.BlockSpec(memory_space=pltpu.VMEM),
        scratch_shapes=[
            pltpu.VMEM((B, D), _BF16),
            pltpu.VMEM((B, HKV, SK, DH), _BF16),
            pltpu.VMEM((B, HKV, SK, DH), _BF16),
            pltpu.VMEM((HKV, DH, SK // 2), _U32),
            pltpu.VMEM((D, HQ * DH), _BF16),
            pltpu.VMEM((HQ * DH, D), _BF16),
            pltpu.VMEM((D, F), _BF16),
            pltpu.VMEM((F, D), _BF16),
            pltpu.VMEM((HKV, _ROWS, DH), _BF16),
            pltpu.VMEM((HKV, _ROWS, DH), _BF16),
            pltpu.VMEM((HKV, _ROWS, SK), _BF16),
            pltpu.VMEM((HKV, _ROWS, DH), _F32),
            pltpu.VMEM((HKV, _ROWS, DH), _F32),
            pltpu.VMEM((HKV, _ROWS, DH), _F32),
            pltpu.VMEM((_ROWS, F), _F32),
            pltpu.VMEM((D // 2, HQ * DH), _U32),
            pltpu.VMEM((HQ * DH // 2, D), _U32),
            pltpu.VMEM((D // 2, F), _U32),
            pltpu.VMEM((F // 2, D), _U32),
            pltpu.VMEM((_FV, D), _F32),
            pltpu.VMEM((_FV, DH), _F32),
            pltpu.VMEM((_FV, D), _F32),
            *[pltpu.VMEM((2 * DH + 8, DH), _U32) for _ in range(_N_COLS)],
            pltpu.SemaphoreType.DMA((_N_SEMS,)),
        ],
        compiler_params=pltpu.CompilerParams(
            vmem_limit_bytes=118 * 1024 * 1024),
    )(A_x.reshape(B, D), A_k_cache, A_v_cache, A_wq, A_wo, B_w1, B_w2)
    return out.reshape(B, SQ, D)
```

```python
import jax
import jax.numpy as jnp
from jax import lax
import jax.experimental.pallas as pl
import jax.experimental.pallas.tpu as pltpu

_BF16 = jnp.bfloat16
_F32 = jnp.float32
_U32 = jnp.uint32
_NT = (((1,), (1,)), ((), ()))
_LN_EPS = 1e-5
_ROWS = 8
_LOG2E = 1.4426950408889634

_TAIL_SPLITS = (6144, 1536, 512)
_N_SEMS = 5
_V1_SPLIT = 5
_FV = 640
_N_COLS = 8

_SCHED = ("mq0 wq1 wq2 wq3 wq4 wq5 wq6 wq7 qa0 qb0 qa1 qb1 pl0 ph0 qa2 qb2 "
          "pl1 ph1 qa3 wo0 tk qb3 pl2 ph2 qa4 wo1 tk qb4 pl3 ph3 qa5 wo2 tk "
          "qb5 pl4 ph4 qa6 wo3 tk qb6 pl5 ph5 qa7 wo4 tk qb7 pl6 ph6 wo5 tk "
          "pl7 ph7 wo6 mo7")


def _kernel_body(dims, x_hbm, k_hbm, v_hbm, wq_hbm, wo_hbm, w1_hbm, w2_hbm,
                 o_ref,
                 x_v, k_v, v_v, kt_v, wq_v, wo_v, w1_v, w2_v,
                 q1_v, q2_v, p_v, linv_v, o_v, csq_v, cs1_v,
                 wqp_v, wop_v, w1p_v, w2p_v, w1t_v, cs1c_v, w2f_v,
                 *rest):
    col_v, sems = rest[:_N_COLS], rest[_N_COLS]
    B, D, HKV, SK, DH, REP, F = dims
    G = REP * DH
    HALF = SK // 2
    HH = HKV // 2
    HL = HKV - 1
    FM = F - _FV
    qscale = (DH ** -0.5) * _LOG2E

    def cp(src, dst, i):
        return pltpu.make_async_copy(src, dst, sems.at[i])

    def kv_cp(hbm, vm, b, h0, h1, i):
        return cp(hbm.at[b, pl.ds(h0, h1 - h0)], vm.at[b, pl.ds(h0, h1 - h0)], i)

    tail_offs = []
    off = 0
    for n in _TAIL_SPLITS:
        tail_offs.append((off, n))
        off += n
    assert off == SK and len(tail_offs) == 3

    c_x = lambda: cp(x_hbm, x_v, 0)
    c_wq = lambda: cp(wq_hbm, wq_v, 0)
    c_wo = lambda: cp(wo_hbm, wo_v, 1)
    c_w1 = lambda: cp(w1_hbm, w1_v, 1)
    c_w2 = lambda: cp(w2_hbm, w2_v, 1)
    c_k0 = lambda: kv_cp(k_hbm, k_v, 0, 0, HKV, 2)
    c_v0a = lambda: kv_cp(v_hbm, v_v, 0, 0, HH, 3)
    c_v0b = lambda: kv_cp(v_hbm, v_v, 0, HH, HKV, 4)
    c_k1a = lambda: kv_cp(k_hbm, k_v, 1, 0, HH, 0)
    c_k1b = lambda: kv_cp(k_hbm, k_v, 1, HH, HKV, 1)
    c_v1a = lambda: kv_cp(v_hbm, v_v, 1, 0, _V1_SPLIT, 2)
    c_v1b = lambda: kv_cp(v_hbm, v_v, 1, _V1_SPLIT, HL, 3)

    def c_vt(i):
        o, n = tail_offs[i]
        return cp(v_hbm.at[1, HL, pl.ds(o, n)], v_v.at[1, HL, pl.ds(o, n)],
                  (4, 0, 1)[i])

    for c in (c_x, c_wq, c_wo, c_w1, c_w2, c_k0, c_v0a, c_v0b):
        c().start()

    row = lax.broadcasted_iota(jnp.int32, (_ROWS, DH), 0)
    row_in_grp = row % REP
    lo_rows = row < REP
    row_d = lax.broadcasted_iota(jnp.int32, (_ROWS, D), 0)

    def dot(a, b):
        return jnp.dot(a, b, preferred_element_type=_F32)

    def pack(x):
        return pltpu.bitcast(x, _U32)

    def unpack(x):
        return pltpu.bitcast(x, _BF16)

    vu_v = v_v.bitcast(_U32)

    def ln_stats(x):
        m = jnp.mean(x, axis=-1, keepdims=True)
        xc = x - m
        var = jnp.mean(xc * xc, axis=-1, keepdims=True)
        return m, xc, lax.rsqrt(var + _LN_EPS)

    def ln_stats1(x):
        m = jnp.mean(x, axis=-1, keepdims=True)
        m2 = jnp.mean(x * x, axis=-1, keepdims=True)
        var = jnp.maximum(m2 - m * m, 0.0)
        return m, x - m, lax.rsqrt(var + _LN_EPS)

    def layernorm(x):
        _, xc, r = ln_stats(x)
        return xc * r

    def pick_heads(res):
        q = res[:, 0:DH]
        for j in range(1, REP):
            q = jnp.where(row_in_grp == j, res[:, j * DH:(j + 1) * DH], q)
        return q

    def softmax_p(s):
        m = jnp.max(s, axis=-1, keepdims=True)
        p = jnp.exp2(s - m)
        l = jnp.sum(p, axis=-1, keepdims=True)
        return p.astype(_BF16), m, l

    def block_diag(o):
        parts = [jnp.where(row_in_grp == j, o, 0.0) for j in range(REP)]
        return jnp.concatenate(parts, axis=1).astype(_BF16)

    def sum_rows(acc, lo, n):
        if n < _ROWS:
            valid = jnp.logical_and(row_d >= lo, row_d < lo + n)
            acc = jnp.where(valid, acc, 0.0)
        r = jnp.sum(acc, axis=0, keepdims=True)
        return jnp.broadcast_to(r, (_ROWS, D))

    def silu_half(hh):
        return hh + hh * jnp.tanh(hh)

    def ffn(x):
        xn = layernorm(x).astype(_BF16)
        h = silu_half(0.5 * dot(xn, w1_v[...]))
        return x + dot(h.astype(_BF16), w2_v[...])

    def q_all(x, q_ref):
        xn = layernorm(x).astype(_BF16)
        res = dot(xn, wq_v[...])
        for g in range(HKV):
            q_ref[g] = (pick_heads(res[:, g * G:(g + 1) * G]) * qscale).astype(_BF16)

    def wo_all(lo):
        lhs = jnp.concatenate([block_diag(o_v[g]) for g in range(HKV)], axis=1)
        return sum_rows(dot(lhs, wo_v[...]), lo, REP)

    c_x().wait()
    c_wq().wait()
    c_k1a().start()
    xin = x_v[...].astype(_F32)
    x0 = jnp.broadcast_to(xin[0:1, :], (_ROWS, D))
    x1 = jnp.broadcast_to(xin[1:2, :], (_ROWS, D))
    x01 = jnp.where(row_d < REP, x0, x1)
    q_all(x01, q1_v)

    ones = jnp.ones((_ROWS, D), _BF16)
    csq = dot(ones, wq_v[...])
    for g in range(HKV):
        csq_v[g] = pick_heads(csq[:, g * G:(g + 1) * G])
    c_wo().wait()
    c_w1().wait()
    c_w2().wait()
    c_k1b().start()
    cs1_v[...] = dot(ones, w1_v[...])
    for src, dst in ((wq_v, wqp_v), (wo_v, wop_v), (w1_v, w1p_v), (w2_v, w2p_v)):
        def pack_rows(i, carry, src=src, dst=dst):
            r0 = pl.multiple_of(i * 64, 64)
            r1 = pl.multiple_of(i * 32, 32)
            dst[pl.ds(r1, 32), :] = pack(src[pl.ds(r0, 64), :])
            return carry
        lax.fori_loop(0, src.shape[0] // 64, pack_rows, 0)
    w1t = w1_v[:, FM:F].astype(_F32).T
    w1t_v[...] = w1t
    w2f_v[...] = w2_v[FM:F, :].astype(_F32)
    cs1c_v[...] = jnp.broadcast_to(jnp.sum(w1t, axis=1, keepdims=True), (_FV, DH))
    for c in col_v:
        c[2 * DH:2 * DH + 8, :] = jnp.zeros((8, DH), _U32)

    c_k0().wait()
    c_v1a().start()

    def qk0_head(h, carry):
        s = lax.dot_general(q1_v[h], k_v[0, h], _NT, preferred_element_type=_F32)
        p, _, l = softmax_p(s)
        p_v[h] = p
        linv_v[h] = jnp.broadcast_to(1.0 / l, (_ROWS, DH))
        return carry
    lax.fori_loop(0, HKV, qk0_head, 0)

    def pv0_head(h, carry):
        @pl.when(h == 0)
        def _():
            c_v0a().wait()
            c_v1b().start()

        @pl.when(h == HH)
        def _():
            c_v0b().wait()
            c_vt(0).start()
        o_v[h] = dot(p_v[h], v_v[0, h]) * linv_v[h]
        return carry
    lax.fori_loop(0, HKV, pv0_head, 0)

    x0 = x0 + wo_all(0)
    x0 = ffn(x0)
    q_all(x0, q2_v)

    def attn0_head(h, carry):
        s = lax.dot_general(q2_v[h], k_v[0, h], _NT, preferred_element_type=_F32)
        p, _, l = softmax_p(s)
        o_v[h] = dot(p, v_v[0, h]) * (1.0 / l)
        return carry
    lax.fori_loop(0, HKV, attn0_head, 0)
    x0 = x0 + wo_all(0)
    x0 = ffn(x0)

    eye = (lax.broadcasted_iota(jnp.int32, (DH, DH), 0)
           == lax.broadcasted_iota(jnp.int32, (DH, DH), 1)).astype(_BF16)

    def qkt_head(h, carry):
        @pl.when(h == 0)
        def _():
            c_k1a().wait()
            c_vt(1).start()

        @pl.when(h == HH)
        def _():
            c_k1b().wait()
            c_vt(2).start()
        q = q1_v[h]
        lhs = jnp.concatenate([eye, q, q], axis=0)
        r = lax.dot_general(lhs, k_v[1, h], _NT, preferred_element_type=_F32)
        kt_v[h, 0:DH // 2, :] = pack(r[:DH, :HALF].astype(_BF16))
        kt_v[h, DH // 2:DH, :] = pack(r[:DH, HALF:].astype(_BF16))
        p, _, l = softmax_p(r[DH:DH + _ROWS])
        p_v[h] = p
        linv_v[h] = jnp.broadcast_to(1.0 / l, (_ROWS, DH))
        return carry + h
    zero = lax.fori_loop(0, HKV, qkt_head, 0) - (HKV * (HKV - 1)) // 2
    zero = jnp.clip(zero, 0, 1)

    def pv1_head(h, acc):
        @pl.when(h == 0)
        def _():
            c_v1a().wait()

        @pl.when(h == _V1_SPLIT)
        def _():
            c_v1b().wait()
        o = dot(p_v[h], v_v[1, h]) * linv_v[h]
        w = wo_v[pl.ds(pl.multiple_of(h * G, G), G), :]
        return acc + dot(block_diag(o), w)
    acc = lax.fori_loop(0, HL, pv1_head, jnp.zeros((_ROWS, D), _F32))

    _, x1c, _ = ln_stats(x1)
    upd = sum_rows(acc, REP, REP)
    y_part = x1c + upd
    x_part = x1 + upd

    def ffn_tail(x, y):
        yb = y.astype(_BF16)
        yf = yb.astype(_F32)
        m, yc, r = ln_stats1(yf)
        rh = 0.5 * r
        hh = (dot(yb, unpack(w1p_v[:, 0:FM])) - m * cs1_v[:, 0:FM]) * rh
        upd = dot(silu_half(hh).astype(_BF16), unpack(w2p_v[0:FM // 2, :]))
        a = None
        for nb in range(_FV // 8):
            t = w1t_v[nb * 8:(nb + 1) * 8, :] * yf
            t = (t[:, 0:DH] + t[:, DH:2 * DH]) + (t[:, 2 * DH:3 * DH] + t[:, 3 * DH:])
            hs = jnp.sum(t, axis=1, keepdims=True)
            hc = silu_half((hs - m * cs1c_v[nb * 8:(nb + 1) * 8, :]) * rh)
            u = w2f_v[nb * 8:(nb + 1) * 8, :] * jnp.concatenate([hc] * (D // DH), axis=1)
            a = u if a is None else a + u
        upd = upd + sum_rows(a, 0, _ROWS)
        return x + upd, yc + upd

    for i, (o_, n) in enumerate(tail_offs):
        c_vt(i).wait()
        o = dot(p_v[HL, :, o_:o_ + n], unpack(vu_v[1, HL, o_ // 2:(o_ + n) // 2, :]))
        if i > 0:
            o = o + o_v[HL]
        if i + 1 < len(tail_offs):
            o_v[HL] = o
    o = o * linv_v[HL]
    upd = sum_rows(dot(block_diag(o), unpack(wop_v[HL * G // 2:(HL + 1) * G // 2, :])),
                   REP, REP)
    x1, y = ffn_tail(x_part + upd, y_part + upd)

    def to_col(rows, col_ref):
        u = [pltpu.bitcast(jnp.broadcast_to(r_, (_ROWS, DH)), _U32) for r_ in rows]
        pk = [(u[0] >> 16) | u[1], (u[2] >> 16) | u[3]]
        rep = jnp.concatenate(
            [jnp.broadcast_to(p_[0:1, :], (DH, DH)) for p_ in pk], axis=1)
        col_ref[0:2 * DH, :] = rep.T

    def col_pair(col_ref, i):
        u = col_ref[pl.ds(pl.multiple_of((zero + i) * 8, 8), 8), :]
        return (pltpu.bitcast(u << 16, _F32),
                pltpu.bitcast(u & jnp.uint32(0xFFFF0000), _F32))

    toks = []

    def gate(x):
        while toks:
            x = jnp.where(zero != 0, toks.pop().astype(x.dtype), x)
        return x

    last = [None] * 4

    def vpu_matvec(col_ref, wp_ref, r0, c0):
        accs = [None] * 4
        for p_ in range(2):
            for kb in range(DH // 16):
                cks = [col_pair(col_ref, p_ * (DH // 8) + kb * 2 + sub)
                       for sub in range(2)]
                for hl in range(2):
                    rr = (r0 + (2 * p_ + hl) * DH) // 2 + kb * 8
                    ws = [unpack(wp_ref[rr:rr + 8, c0 + j * DH:c0 + (j + 1) * DH]
                                 ).astype(_F32) for j in range(4)]
                    for sub in range(2):
                        for j in range(4):
                            t = ws[j][sub * 8:(sub + 1) * 8, :] * cks[sub][hl]
                            accs[j] = t if accs[j] is None else accs[j] + t
        last[:] = accs
        return accs

    def fold_rows(a):
        def fold(x, y_, sh):
            msk = (row % (2 * sh)) < sh
            if 2 * sh == _ROWS:
                return (jnp.where(msk, x, y_)
                        + pltpu.roll(jnp.where(msk, y_, x), sh, axis=0))
            return jnp.where(msk, x + pltpu.roll(x, _ROWS - sh, axis=0),
                             y_ + pltpu.roll(y_, sh, axis=0))
        b = [fold(a[i], a[i + 4], 4) for i in range(4)]
        c = [fold(b[i], b[i + 2], 2) for i in range(2)]
        return fold(c[0], c[1], 1)

    yb = y.astype(_BF16)
    yf = yb.astype(_F32)
    m, yc, r = ln_stats1(yf)
    rq = r * qscale
    to_col([yf[0:1, j * DH:(j + 1) * DH] for j in range(D // DH)], col_v[0])
    qb, sm, ps, oh, os_ = {}, {}, {}, {}, {}
    st = {"mx": None, "vp": None}

    def finish_q(g, res):
        qb[g] = ((res - m * csq_v[g]) * rq).astype(_BF16)

    def t_mq(g):
        finish_q(g, pick_heads(dot(yb, unpack(wqp_v[:, g * G:(g + 1) * G]))))

    def t_wq(g):
        accs = vpu_matvec(col_v[0], wqp_v, 0, g * G)
        finish_q(g, fold_rows(accs + accs))

    def t_tk():
        toks.append((last[0] + last[1]) + (last[2] + last[3]))

    def t_q(g, part):
        q = gate(qb[g])
        zq = jnp.zeros_like(q)
        q2 = jnp.concatenate(
            [jnp.where(lo_rows, q, zq), jnp.where(lo_rows, zq, q)], axis=1)
        c0 = part * (HALF // 2)
        sm.setdefault(g, []).append(dot(q2, unpack(kt_v[g, :, c0:c0 + HALF // 2])))

    def t_sm(g):
        p, mx, l = softmax_p(jnp.concatenate(sm.pop(g), axis=1))
        mx = jnp.broadcast_to(mx, (_ROWS, DH))
        l = jnp.broadcast_to(l, (_ROWS, DH))
        mx_all = jnp.maximum(mx, pltpu.roll(mx, REP, axis=0))
        a = jnp.exp2(mx - mx_all)
        al = a * l
        ps[g] = (p, a / (al + pltpu.roll(al, REP, axis=0)))

    def t_p(g, part):
        if g not in ps:
            t_sm(g)
        p, c = ps[g]
        if toks:
            tk = list(toks)
            pieces = []
            for i in range(4):
                toks[:] = tk
                pieces.append(gate(p[:, i * DH:(i + 1) * DH]))
            p = jnp.concatenate(pieces + [p[:, 4 * DH:]], axis=1)
        o = dot(p, unpack(vu_v[1, g, part * (HALF // 2):(part + 1) * (HALF // 2), :]))
        if part == 0:
            oh[g] = o
        else:
            os_[g] = jnp.where(lo_rows, oh.pop(g), o) * c

    def t_mo(g):
        part = dot(block_diag(gate(os_.pop(g))),
                   unpack(wop_v[g * G // 2:(g + 1) * G // 2, :]))
        st["mx"] = part if st["mx"] is None else part + st["mx"]

    def t_wo(g):
        o = os_.pop(g)
        o4 = (o + pltpu.roll(o, REP, axis=0)).astype(_BF16).astype(_F32)
        to_col([o4[j:j + 1, :] for j in range(REP)], col_v[1 + g])
        part = jnp.concatenate(vpu_matvec(col_v[1 + g], wop_v, g * G, 0), axis=1)
        st["vp"] = part if st["vp"] is None else st["vp"] + part

    tasks = {"mq": t_mq, "wq": t_wq, "tk": t_tk, "mo": t_mo, "wo": t_wo,
             "qa": lambda g: t_q(g, 0), "qb": lambda g: t_q(g, 1),
             "pl": lambda g: t_p(g, 0), "ph": lambda g: t_p(g, 1)}
    for item in _SCHED.split():
        tasks[item[:2]](*[int(c) for c in item[2:]])
    assert not os_ and not toks
    upd = sum_rows(st["mx"] + st["vp"], 0, _ROWS)
    x1, _ = ffn_tail(x1 + upd, yc + upd)
    out = jnp.where(row_d < 1, x0, x1)
    o_ref[...] = out[0:B, :].astype(o_ref.dtype)


@jax.jit
def pallas_interleave_layers__gqa_block_cached__dense_activation_silu__decode_kernel(
    A_x: jax.Array,
    A_k_cache: jax.Array,
    A_v_cache: jax.Array,
    A_wq: jax.Array,
    A_wo: jax.Array,
    B_x: jax.Array,
    B_w1: jax.Array,
    B_w2: jax.Array,
):
    del B_x
    B, SQ, D = A_x.shape
    _, HKV, SK, DH = A_k_cache.shape
    HQ = A_wq.shape[1] // DH
    REP = HQ // HKV
    F = B_w1.shape[1]
    assert B == 2 and SQ == 1 and 2 * REP == _ROWS and HKV == 8
    assert D == REP * DH and DH == 128
    dims = (B, D, HKV, SK, DH, REP, F)

    def kernel(*refs):
        _kernel_body(dims, *refs)

    any_spec = pl.BlockSpec(memory_space=pl.ANY)
    out = pl.pallas_call(
        kernel,
        out_shape=jax.ShapeDtypeStruct((B, D), A_x.dtype),
        in_specs=[any_spec] * 7,
        out_specs=pl.BlockSpec(memory_space=pltpu.VMEM),
        scratch_shapes=[
            pltpu.VMEM((B, D), _BF16),
            pltpu.VMEM((B, HKV, SK, DH), _BF16),
            pltpu.VMEM((B, HKV, SK, DH), _BF16),
            pltpu.VMEM((HKV, DH, SK // 2), _U32),
            pltpu.VMEM((D, HQ * DH), _BF16),
            pltpu.VMEM((HQ * DH, D), _BF16),
            pltpu.VMEM((D, F), _BF16),
            pltpu.VMEM((F, D), _BF16),
            pltpu.VMEM((HKV, _ROWS, DH), _BF16),
            pltpu.VMEM((HKV, _ROWS, DH), _BF16),
            pltpu.VMEM((HKV, _ROWS, SK), _BF16),
            pltpu.VMEM((HKV, _ROWS, DH), _F32),
            pltpu.VMEM((HKV, _ROWS, DH), _F32),
            pltpu.VMEM((HKV, _ROWS, DH), _F32),
            pltpu.VMEM((_ROWS, F), _F32),
            pltpu.VMEM((D // 2, HQ * DH), _U32),
            pltpu.VMEM((HQ * DH // 2, D), _U32),
            pltpu.VMEM((D // 2, F), _U32),
            pltpu.VMEM((F // 2, D), _U32),
            pltpu.VMEM((_FV, D), _F32),
            pltpu.VMEM((_FV, DH), _F32),
            pltpu.VMEM((_FV, D), _F32),
            *[pltpu.VMEM((2 * DH + 8, DH), _U32) for _ in range(_N_COLS)],
            pltpu.SemaphoreType.DMA((_N_SEMS,)),
        ],
        compiler_params=pltpu.CompilerParams(
            vmem_limit_bytes=118 * 1024 * 1024),
    )(A_x.reshape(B, D), A_k_cache, A_v_cache, A_wq, A_wo, B_w1, B_w2)
    return out.reshape(B, SQ, D)
```

```python
import jax
import jax.numpy as jnp
from jax import lax
import jax.experimental.pallas as pl
import jax.experimental.pallas.tpu as pltpu

_BF16 = jnp.bfloat16
_F32 = jnp.float32
_U32 = jnp.uint32
_NT = (((1,), (1,)), ((), ()))
_LN_EPS = 1e-5
_ROWS = 8
_LOG2E = 1.4426950408889634

_TAIL_SPLITS = (6144, 1536, 512)
_N_SEMS = 5
_V1_SPLIT = 5
_FV = 768
_NBT = 40
_N_COLS = 8

_SCHED = ("mq0 wq1 wq2 wq3 wq4 wq5 wq6 wq7 qa0 qb0 qa1 qb1 pl0 ph0 qa2 qb2 "
          "pl1 ph1 qa3 wo0 tk qb3 pl2 ph2 qa4 wo1 tk qb4 pl3 ph3 qa5 wo2 tk "
          "qb5 pl4 ph4 qa6 wo3 tk qb6 pl5 ph5 qa7 wo4 tk qb7 pl6 ph6 wo5 tk "
          "pl7 ph7 wo6 mo7")


def _kernel_body(dims, x_hbm, k_hbm, v_hbm, wq_hbm, wo_hbm, w1_hbm, w2_hbm,
                 o_ref,
                 x_v, k_v, v_v, kt_v, wq_v, wo_v, w1_v, w2_v,
                 q1_v, q2_v, p_v, linv_v, o_v, csq_v, cs1_v,
                 wqp_v, wop_v, w1p_v, w2p_v, w1t_v, cs1c_v, w2f_v,
                 *rest):
    col_v, sems = rest[:_N_COLS], rest[_N_COLS]
    B, D, HKV, SK, DH, REP, F = dims
    G = REP * DH
    HALF = SK // 2
    HH = HKV // 2
    HL = HKV - 1
    FM = F - _FV
    qscale = (DH ** -0.5) * _LOG2E

    def cp(src, dst, i):
        return pltpu.make_async_copy(src, dst, sems.at[i])

    def kv_cp(hbm, vm, b, h0, h1, i):
        return cp(hbm.at[b, pl.ds(h0, h1 - h0)], vm.at[b, pl.ds(h0, h1 - h0)], i)

    tail_offs = []
    off = 0
    for n in _TAIL_SPLITS:
        tail_offs.append((off, n))
        off += n
    assert off == SK and len(tail_offs) == 3

    c_x = lambda: cp(x_hbm, x_v, 0)
    c_wq = lambda: cp(wq_hbm, wq_v, 0)
    c_wo = lambda: cp(wo_hbm, wo_v, 1)
    c_w1 = lambda: cp(w1_hbm, w1_v, 1)
    c_w2 = lambda: cp(w2_hbm, w2_v, 1)
    c_k0 = lambda: kv_cp(k_hbm, k_v, 0, 0, HKV, 2)
    c_v0a = lambda: kv_cp(v_hbm, v_v, 0, 0, HH, 3)
    c_v0b = lambda: kv_cp(v_hbm, v_v, 0, HH, HKV, 4)
    c_k1a = lambda: kv_cp(k_hbm, k_v, 1, 0, HH, 0)
    c_k1b = lambda: kv_cp(k_hbm, k_v, 1, HH, HKV, 1)
    c_v1a = lambda: kv_cp(v_hbm, v_v, 1, 0, _V1_SPLIT, 2)
    c_v1b = lambda: kv_cp(v_hbm, v_v, 1, _V1_SPLIT, HL, 3)

    def c_vt(i):
        o, n = tail_offs[i]
        return cp(v_hbm.at[1, HL, pl.ds(o, n)], v_v.at[1, HL, pl.ds(o, n)],
                  (4, 0, 1)[i])

    for c in (c_x, c_wq, c_wo, c_w1, c_w2, c_k0, c_v0a, c_v0b):
        c().start()

    row = lax.broadcasted_iota(jnp.int32, (_ROWS, DH), 0)
    lane = lax.broadcasted_iota(jnp.int32, (_ROWS, DH), 1)
    row_in_grp = row % REP
    lo_rows = row < REP
    row_d = lax.broadcasted_iota(jnp.int32, (_ROWS, D), 0)

    def dot(a, b):
        return jnp.dot(a, b, preferred_element_type=_F32)

    def pack(x):
        return pltpu.bitcast(x, _U32)

    def unpack(x):
        return pltpu.bitcast(x, _BF16)

    vu_v = v_v.bitcast(_U32)

    def ln_stats(x):
        m = jnp.mean(x, axis=-1, keepdims=True)
        xc = x - m
        var = jnp.mean(xc * xc, axis=-1, keepdims=True)
        return m, xc, lax.rsqrt(var + _LN_EPS)

    def ln_stats1(x):
        m = jnp.mean(x, axis=-1, keepdims=True)
        m2 = jnp.mean(x * x, axis=-1, keepdims=True)
        var = jnp.maximum(m2 - m * m, 0.0)
        return m, x - m, lax.rsqrt(var + _LN_EPS)

    def layernorm(x):
        _, xc, r = ln_stats(x)
        return xc * r

    def pick_heads(res):
        q = res[:, 0:DH]
        for j in range(1, REP):
            q = jnp.where(row_in_grp == j, res[:, j * DH:(j + 1) * DH], q)
        return q

    def softmax_p(s):
        m = jnp.max(s, axis=-1, keepdims=True)
        p = jnp.exp2(s - m)
        l = jnp.sum(p, axis=-1, keepdims=True)
        return p.astype(_BF16), m, l

    def block_diag(o):
        parts = [jnp.where(row_in_grp == j, o, 0.0) for j in range(REP)]
        return jnp.concatenate(parts, axis=1).astype(_BF16)

    def sum_rows(acc, lo, n):
        if n < _ROWS:
            valid = jnp.logical_and(row_d >= lo, row_d < lo + n)
            acc = jnp.where(valid, acc, 0.0)
        r = jnp.sum(acc, axis=0, keepdims=True)
        return jnp.broadcast_to(r, (_ROWS, D))

    def silu_half(hh):
        return hh + hh * jnp.tanh(hh)

    def ffn(x):
        xn = layernorm(x).astype(_BF16)
        h = silu_half(0.5 * dot(xn, w1_v[...]))
        return x + dot(h.astype(_BF16), w2_v[...])

    def q_all(x, q_ref):
        xn = layernorm(x).astype(_BF16)
        res = dot(xn, wq_v[...])
        for g in range(HKV):
            q_ref[g] = (pick_heads(res[:, g * G:(g + 1) * G]) * qscale).astype(_BF16)

    def wo_all(lo):
        lhs = jnp.concatenate([block_diag(o_v[g]) for g in range(HKV)], axis=1)
        return sum_rows(dot(lhs, wo_v[...]), lo, REP)

    c_x().wait()
    c_wq().wait()
    c_k1a().start()
    xin = x_v[...].astype(_F32)
    x0 = jnp.broadcast_to(xin[0:1, :], (_ROWS, D))
    x1 = jnp.broadcast_to(xin[1:2, :], (_ROWS, D))
    x01 = jnp.where(row_d < REP, x0, x1)
    q_all(x01, q1_v)

    ones = jnp.ones((_ROWS, D), _BF16)
    csq = dot(ones, wq_v[...])
    for g in range(HKV):
        csq_v[g] = pick_heads(csq[:, g * G:(g + 1) * G])
    c_wo().wait()
    c_w1().wait()
    c_w2().wait()
    c_k1b().start()
    cs1_v[...] = dot(ones, w1_v[...])
    for src, dst in ((wq_v, wqp_v), (wo_v, wop_v), (w1_v, w1p_v), (w2_v, w2p_v)):
        def pack_rows(i, carry, src=src, dst=dst):
            r0 = pl.multiple_of(i * 64, 64)
            r1 = pl.multiple_of(i * 32, 32)
            dst[pl.ds(r1, 32), :] = pack(src[pl.ds(r0, 64), :])
            return carry
        lax.fori_loop(0, src.shape[0] // 64, pack_rows, 0)
    w1t = w1_v[:, FM:F].astype(_F32).T
    w1t_v[...] = w1t
    w2f_v[...] = w2_v[FM:F, :].astype(_F32)
    w1s = jnp.broadcast_to(jnp.sum(w1t, axis=1, keepdims=True), (_FV, DH))
    ccat = jnp.zeros((_ROWS, DH), _F32)
    for nb in range(_NBT):
        ccat = jnp.where(lane == nb, w1s[nb * 8:(nb + 1) * 8, :], ccat)
    cs1c_v[0:_FV, :] = w1s
    cs1c_v[_FV:_FV + 8, :] = ccat
    for c in col_v:
        c[2 * DH:2 * DH + 8, :] = jnp.zeros((8, DH), _U32)

    c_k0().wait()
    c_v1a().start()

    def qk0_head(h, carry):
        s = lax.dot_general(q1_v[h], k_v[0, h], _NT, preferred_element_type=_F32)
        p, _, l = softmax_p(s)
        p_v[h] = p
        linv_v[h] = jnp.broadcast_to(1.0 / l, (_ROWS, DH))
        return carry
    lax.fori_loop(0, HKV, qk0_head, 0)

    def pv0_head(h, carry):
        @pl.when(h == 0)
        def _():
            c_v0a().wait()
            c_v1b().start()

        @pl.when(h == HH)
        def _():
            c_v0b().wait()
            c_vt(0).start()
        o_v[h] = dot(p_v[h], v_v[0, h]) * linv_v[h]
        return carry
    lax.fori_loop(0, HKV, pv0_head, 0)

    x0 = x0 + wo_all(0)
    x0 = ffn(x0)
    q_all(x0, q2_v)

    def attn0_head(h, carry):
        s = lax.dot_general(q2_v[h], k_v[0, h], _NT, preferred_element_type=_F32)
        p, _, l = softmax_p(s)
        o_v[h] = dot(p, v_v[0, h]) * (1.0 / l)
        return carry
    lax.fori_loop(0, HKV, attn0_head, 0)
    x0 = x0 + wo_all(0)
    x0 = ffn(x0)

    eye = (lax.broadcasted_iota(jnp.int32, (DH, DH), 0)
           == lax.broadcasted_iota(jnp.int32, (DH, DH), 1)).astype(_BF16)

    def qkt_head(h, carry):
        @pl.when(h == 0)
        def _():
            c_k1a().wait()
            c_vt(1).start()

        @pl.when(h == HH)
        def _():
            c_k1b().wait()
            c_vt(2).start()
        q = q1_v[h]
        lhs = jnp.concatenate([eye, q, q], axis=0)
        r = lax.dot_general(lhs, k_v[1, h], _NT, preferred_element_type=_F32)
        kt_v[h, 0:DH // 2, :] = pack(r[:DH, :HALF].astype(_BF16))
        kt_v[h, DH // 2:DH, :] = pack(r[:DH, HALF:].astype(_BF16))
        p, _, l = softmax_p(r[DH:DH + _ROWS])
        p_v[h] = p
        linv_v[h] = jnp.broadcast_to(1.0 / l, (_ROWS, DH))
        return carry + h
    zero = lax.fori_loop(0, HKV, qkt_head, 0) - (HKV * (HKV - 1)) // 2
    zero = jnp.clip(zero, 0, 1)

    def pv1_head(h, acc):
        @pl.when(h == 0)
        def _():
            c_v1a().wait()

        @pl.when(h == _V1_SPLIT)
        def _():
            c_v1b().wait()
        o = dot(p_v[h], v_v[1, h]) * linv_v[h]
        w = wo_v[pl.ds(pl.multiple_of(h * G, G), G), :]
        return acc + dot(block_diag(o), w)
    acc = lax.fori_loop(0, HL, pv1_head, jnp.zeros((_ROWS, D), _F32))

    _, x1c, _ = ln_stats(x1)
    upd = sum_rows(acc, REP, REP)
    y_part = x1c + upd
    x_part = x1 + upd

    def ffn_tail(x, y):
        yb = y.astype(_BF16)
        yf = yb.astype(_F32)
        m, yc, r = ln_stats1(yf)
        rh = 0.5 * r
        hh = (dot(yb, unpack(w1p_v[:, 0:FM])) - m * cs1_v[:, 0:FM]) * rh
        upd = dot(silu_half(hh).astype(_BF16), unpack(w2p_v[0:FM // 2, :]))
        nblk = _FV // 8
        hs = []
        for nb in range(nblk):
            t = w1t_v[nb * 8:(nb + 1) * 8, :] * yf
            t = (t[:, 0:DH] + t[:, DH:2 * DH]) + (t[:, 2 * DH:3 * DH] + t[:, 3 * DH:])
            hs.append(jnp.broadcast_to(jnp.sum(t, axis=1, keepdims=True), (_ROWS, DH)))
        hcat = hs[0]
        for nb in range(1, _NBT):
            hcat = jnp.where(lane == nb, hs[nb], hcat)
        hcat = silu_half((hcat - m * cs1c_v[_FV:_FV + 8, :]) * rh)
        a = None
        for nb in list(range(_NBT, nblk)) + list(range(_NBT)):
            if nb < _NBT:
                hc = jnp.broadcast_to(hcat[:, nb:nb + 1], (_ROWS, DH))
            else:
                hc = silu_half((hs[nb] - m * cs1c_v[nb * 8:(nb + 1) * 8, :]) * rh)
            u = w2f_v[nb * 8:(nb + 1) * 8, :] * jnp.concatenate([hc] * (D // DH), axis=1)
            a = u if a is None else a + u
        upd = upd + sum_rows(a, 0, _ROWS)
        return x + upd, yc + upd

    for i, (o_, n) in enumerate(tail_offs):
        c_vt(i).wait()
        o = dot(p_v[HL, :, o_:o_ + n], unpack(vu_v[1, HL, o_ // 2:(o_ + n) // 2, :]))
        if i > 0:
            o = o + o_v[HL]
        if i + 1 < len(tail_offs):
            o_v[HL] = o
    o = o * linv_v[HL]
    upd = sum_rows(dot(block_diag(o), unpack(wop_v[HL * G // 2:(HL + 1) * G // 2, :])),
                   REP, REP)
    x1, y = ffn_tail(x_part + upd, y_part + upd)

    def to_col(rows, col_ref):
        u = [pltpu.bitcast(jnp.broadcast_to(r_, (_ROWS, DH)), _U32) for r_ in rows]
        pk = [(u[0] >> 16) | u[1], (u[2] >> 16) | u[3]]
        rep = jnp.concatenate(
            [jnp.broadcast_to(p_[0:1, :], (DH, DH)) for p_ in pk], axis=1)
        col_ref[0:2 * DH, :] = rep.T

    def col_pair(col_ref, i):
        u = col_ref[pl.ds(pl.multiple_of((zero + i) * 8, 8), 8), :]
        return (pltpu.bitcast(u << 16, _F32),
                pltpu.bitcast(u & jnp.uint32(0xFFFF0000), _F32))

    toks = []

    def gate(x):
        while toks:
            x = jnp.where(zero != 0, toks.pop().astype(x.dtype), x)
        return x

    last = [None] * 4

    def vpu_matvec(col_ref, wp_ref, r0, c0):
        accs = [None] * 4
        for p_ in range(2):
            for kb in range(DH // 16):
                cks = [col_pair(col_ref, p_ * (DH // 8) + kb * 2 + sub)
                       for sub in range(2)]
                for hl in range(2):
                    rr = (r0 + (2 * p_ + hl) * DH) // 2 + kb * 8
                    ws = [unpack(wp_ref[rr:rr + 8, c0 + j * DH:c0 + (j + 1) * DH]
                                 ).astype(_F32) for j in range(4)]
                    for sub in range(2):
                        for j in range(4):
                            t = ws[j][sub * 8:(sub + 1) * 8, :] * cks[sub][hl]
                            accs[j] = t if accs[j] is None else accs[j] + t
        last[:] = accs
        return accs

    def fold_rows(a):
        def fold(x, y_, sh):
            msk = (row % (2 * sh)) < sh
            if 2 * sh == _ROWS:
                return (jnp.where(msk, x, y_)
                        + pltpu.roll(jnp.where(msk, y_, x), sh, axis=0))
            return jnp.where(msk, x + pltpu.roll(x, _ROWS - sh, axis=0),
                             y_ + pltpu.roll(y_, sh, axis=0))
        b = [fold(a[i], a[i + 4], 4) for i in range(4)]
        c = [fold(b[i], b[i + 2], 2) for i in range(2)]
        return fold(c[0], c[1], 1)

    yb = y.astype(_BF16)
    yf = yb.astype(_F32)
    m, yc, r = ln_stats1(yf)
    rq = r * qscale
    to_col([yf[0:1, j * DH:(j + 1) * DH] for j in range(D // DH)], col_v[0])
    qb, sm, ps, oh, os_ = {}, {}, {}, {}, {}
    st = {"mx": None, "vp": None}

    def finish_q(g, res):
        qb[g] = ((res - m * csq_v[g]) * rq).astype(_BF16)

    def t_mq(g):
        finish_q(g, pick_heads(dot(yb, unpack(wqp_v[:, g * G:(g + 1) * G]))))

    def t_wq(g):
        accs = vpu_matvec(col_v[0], wqp_v, 0, g * G)
        finish_q(g, fold_rows(accs + accs))

    def t_tk():
        toks.append((last[0] + last[1]) + (last[2] + last[3]))

    def t_q(g, part):
        q = gate(qb[g])
        zq = jnp.zeros_like(q)
        q2 = jnp.concatenate(
            [jnp.where(lo_rows, q, zq), jnp.where(lo_rows, zq, q)], axis=1)
        c0 = part * (HALF // 2)
        sm.setdefault(g, []).append(dot(q2, unpack(kt_v[g, :, c0:c0 + HALF // 2])))

    def t_sm(g):
        p, mx, l = softmax_p(jnp.concatenate(sm.pop(g), axis=1))
        mx = jnp.broadcast_to(mx, (_ROWS, DH))
        l = jnp.broadcast_to(l, (_ROWS, DH))
        mx_all = jnp.maximum(mx, pltpu.roll(mx, REP, axis=0))
        a = jnp.exp2(mx - mx_all)
        al = a * l
        ps[g] = (p, a / (al + pltpu.roll(al, REP, axis=0)))

    def t_p(g, part):
        if g not in ps:
            t_sm(g)
        p, c = ps[g]
        if toks:
            tk = list(toks)
            pieces = []
            for i in range(4):
                toks[:] = tk
                pieces.append(gate(p[:, i * DH:(i + 1) * DH]))
            p = jnp.concatenate(pieces + [p[:, 4 * DH:]], axis=1)
        o = dot(p, unpack(vu_v[1, g, part * (HALF // 2):(part + 1) * (HALF // 2), :]))
        if part == 0:
            oh[g] = o
        else:
            os_[g] = jnp.where(lo_rows, oh.pop(g), o) * c

    def t_mo(g):
        part = dot(block_diag(gate(os_.pop(g))),
                   unpack(wop_v[g * G // 2:(g + 1) * G // 2, :]))
        st["mx"] = part if st["mx"] is None else part + st["mx"]

    def t_wo(g):
        o = os_.pop(g)
        o4 = (o + pltpu.roll(o, REP, axis=0)).astype(_BF16).astype(_F32)
        to_col([o4[j:j + 1, :] for j in range(REP)], col_v[1 + g])
        part = jnp.concatenate(vpu_matvec(col_v[1 + g], wop_v, g * G, 0), axis=1)
        st["vp"] = part if st["vp"] is None else st["vp"] + part

    tasks = {"mq": t_mq, "wq": t_wq, "tk": t_tk, "mo": t_mo, "wo": t_wo,
             "qa": lambda g: t_q(g, 0), "qb": lambda g: t_q(g, 1),
             "pl": lambda g: t_p(g, 0), "ph": lambda g: t_p(g, 1)}
    for item in _SCHED.split():
        tasks[item[:2]](*[int(c) for c in item[2:]])
    assert not os_ and not toks
    upd = sum_rows(st["mx"] + st["vp"], 0, _ROWS)
    x1, _ = ffn_tail(x1 + upd, yc + upd)
    out = jnp.where(row_d < 1, x0, x1)
    o_ref[...] = out[0:B, :].astype(o_ref.dtype)


@jax.jit
def pallas_interleave_layers__gqa_block_cached__dense_activation_silu__decode_kernel(
    A_x: jax.Array,
    A_k_cache: jax.Array,
    A_v_cache: jax.Array,
    A_wq: jax.Array,
    A_wo: jax.Array,
    B_x: jax.Array,
    B_w1: jax.Array,
    B_w2: jax.Array,
):
    del B_x
    B, SQ, D = A_x.shape
    _, HKV, SK, DH = A_k_cache.shape
    HQ = A_wq.shape[1] // DH
    REP = HQ // HKV
    F = B_w1.shape[1]
    assert B == 2 and SQ == 1 and 2 * REP == _ROWS and HKV == 8
    assert D == REP * DH and DH == 128
    dims = (B, D, HKV, SK, DH, REP, F)

    def kernel(*refs):
        _kernel_body(dims, *refs)

    any_spec = pl.BlockSpec(memory_space=pl.ANY)
    out = pl.pallas_call(
        kernel,
        out_shape=jax.ShapeDtypeStruct((B, D), A_x.dtype),
        in_specs=[any_spec] * 7,
        out_specs=pl.BlockSpec(memory_space=pltpu.VMEM),
        scratch_shapes=[
            pltpu.VMEM((B, D), _BF16),
            pltpu.VMEM((B, HKV, SK, DH), _BF16),
            pltpu.VMEM((B, HKV, SK, DH), _BF16),
            pltpu.VMEM((HKV, DH, SK // 2), _U32),
            pltpu.VMEM((D, HQ * DH), _BF16),
            pltpu.VMEM((HQ * DH, D), _BF16),
            pltpu.VMEM((D, F), _BF16),
            pltpu.VMEM((F, D), _BF16),
            pltpu.VMEM((HKV, _ROWS, DH), _BF16),
            pltpu.VMEM((HKV, _ROWS, DH), _BF16),
            pltpu.VMEM((HKV, _ROWS, SK), _BF16),
            pltpu.VMEM((HKV, _ROWS, DH), _F32),
            pltpu.VMEM((HKV, _ROWS, DH), _F32),
            pltpu.VMEM((HKV, _ROWS, DH), _F32),
            pltpu.VMEM((_ROWS, F), _F32),
            pltpu.VMEM((D // 2, HQ * DH), _U32),
            pltpu.VMEM((HQ * DH // 2, D), _U32),
            pltpu.VMEM((D // 2, F), _U32),
            pltpu.VMEM((F // 2, D), _U32),
            pltpu.VMEM((_FV, D), _F32),
            pltpu.VMEM((_FV + 8, DH), _F32),
            pltpu.VMEM((_FV, D), _F32),
            *[pltpu.VMEM((2 * DH + 8, DH), _U32) for _ in range(_N_COLS)],
            pltpu.SemaphoreType.DMA((_N_SEMS,)),
        ],
        compiler_params=pltpu.CompilerParams(
            vmem_limit_bytes=118 * 1024 * 1024),
    )(A_x.reshape(B, D), A_k_cache, A_v_cache, A_wq, A_wo, B_w1, B_w2)
    return out.reshape(B, SQ, D)
```

```python
import jax
import jax.numpy as jnp
from jax import lax
import jax.experimental.pallas as pl
import jax.experimental.pallas.tpu as pltpu

_BF16 = jnp.bfloat16
_F32 = jnp.float32
_U32 = jnp.uint32
_NT = (((1,), (1,)), ((), ()))
_LN_EPS = 1e-5
_ROWS = 8
_LOG2E = 1.4426950408889634

_TAIL_SPLITS = (6144, 1536, 512)
_N_SEMS = 5
_V1_SPLIT = 5
_FV = 768
_NBT = 40
_N_COLS = 7

_SCHED = ("mq0 wq1 wq2 wq3 wq4 wq5 wq6 wq7 qa0 qb0 qa1 qb1 pl0 ph0 qa2 qb2 "
          "pl1 ph1 qa3 wo0 tk qb3 pl2 ph2 qa4 wo1 tk qb4 pl3 ph3 qa5 wo2 tk "
          "qb5 pl4 ph4 qa6 wo3 tk qb6 pl5 ph5 qa7 wo4 tk qb7 pl6 ph6 pl7 "
          "wo5 tk ph7 mo6 mo7")


def _kernel_body(dims, x_hbm, k_hbm, v_hbm, wq_hbm, wo_hbm, w1_hbm, w2_hbm,
                 o_ref,
                 x_v, k_v, v_v, kt_v, wq_v, wo_v, w1_v, w2_v,
                 q1_v, q2_v, p_v, linv_v, o_v, csq_v, cs1_v,
                 wqp_v, wop_v, w1p_v, w2p_v, w1t_v, cs1c_v, w2f_v,
                 *rest):
    col_v, sems = rest[:_N_COLS], rest[_N_COLS]
    B, D, HKV, SK, DH, REP, F = dims
    G = REP * DH
    HALF = SK // 2
    HH = HKV // 2
    HL = HKV - 1
    FM = F - _FV
    qscale = (DH ** -0.5) * _LOG2E

    def cp(src, dst, i):
        return pltpu.make_async_copy(src, dst, sems.at[i])

    def kv_cp(hbm, vm, b, h0, h1, i):
        return cp(hbm.at[b, pl.ds(h0, h1 - h0)], vm.at[b, pl.ds(h0, h1 - h0)], i)

    tail_offs = []
    off = 0
    for n in _TAIL_SPLITS:
        tail_offs.append((off, n))
        off += n
    assert off == SK and len(tail_offs) == 3

    c_x = lambda: cp(x_hbm, x_v, 0)
    c_wq = lambda: cp(wq_hbm, wq_v, 0)
    c_wo = lambda: cp(wo_hbm, wo_v, 1)
    c_w1 = lambda: cp(w1_hbm, w1_v, 1)
    c_w2 = lambda: cp(w2_hbm, w2_v, 1)
    c_k0 = lambda: kv_cp(k_hbm, k_v, 0, 0, HKV, 2)
    c_v0a = lambda: kv_cp(v_hbm, v_v, 0, 0, HH, 3)
    c_v0b = lambda: kv_cp(v_hbm, v_v, 0, HH, HKV, 4)
    c_k1a = lambda: kv_cp(k_hbm, k_v, 1, 0, HH, 0)
    c_k1b = lambda: kv_cp(k_hbm, k_v, 1, HH, HKV, 1)
    c_v1a = lambda: kv_cp(v_hbm, v_v, 1, 0, _V1_SPLIT, 2)
    c_v1b = lambda: kv_cp(v_hbm, v_v, 1, _V1_SPLIT, HL, 3)

    def c_vt(i):
        o, n = tail_offs[i]
        return cp(v_hbm.at[1, HL, pl.ds(o, n)], v_v.at[1, HL, pl.ds(o, n)],
                  (4, 0, 1)[i])

    for c in (c_x, c_wq, c_wo, c_w1, c_w2, c_k0, c_v0a, c_v0b):
        c().start()

    row = lax.broadcasted_iota(jnp.int32, (_ROWS, DH), 0)
    lane = lax.broadcasted_iota(jnp.int32, (_ROWS, DH), 1)
    row_in_grp = row % REP
    lo_rows = row < REP
    row_d = lax.broadcasted_iota(jnp.int32, (_ROWS, D), 0)

    def dot(a, b):
        return jnp.dot(a, b, preferred_element_type=_F32)

    def pack(x):
        return pltpu.bitcast(x, _U32)

    def unpack(x):
        return pltpu.bitcast(x, _BF16)

    def ln_stats(x):
        m = jnp.mean(x, axis=-1, keepdims=True)
        xc = x - m
        var = jnp.mean(xc * xc, axis=-1, keepdims=True)
        return m, xc, lax.rsqrt(var + _LN_EPS)

    def ln_stats1(x):
        m = jnp.mean(x, axis=-1, keepdims=True)
        m2 = jnp.mean(x * x, axis=-1, keepdims=True)
        var = jnp.maximum(m2 - m * m, 0.0)
        return m, x - m, lax.rsqrt(var + _LN_EPS)

    def layernorm(x):
        _, xc, r = ln_stats(x)
        return xc * r

    def pick_heads(res):
        q = res[:, 0:DH]
        for j in range(1, REP):
            q = jnp.where(row_in_grp == j, res[:, j * DH:(j + 1) * DH], q)
        return q

    def softmax_p(s):
        m = jnp.max(s, axis=-1, keepdims=True)
        p = jnp.exp2(s - m)
        l = jnp.sum(p, axis=-1, keepdims=True)
        return p.astype(_BF16), m, l

    def block_diag(o):
        parts = [jnp.where(row_in_grp == j, o, 0.0) for j in range(REP)]
        return jnp.concatenate(parts, axis=1).astype(_BF16)

    def sum_rows(acc, lo, n):
        if n < _ROWS:
            valid = jnp.logical_and(row_d >= lo, row_d < lo + n)
            acc = jnp.where(valid, acc, 0.0)
        r = jnp.sum(acc, axis=0, keepdims=True)
        return jnp.broadcast_to(r, (_ROWS, D))

    def silu_half(hh):
        return hh + hh * jnp.tanh(hh)

    def ffn(x):
        xn = layernorm(x).astype(_BF16)
        h = silu_half(0.5 * dot(xn, w1_v[...]))
        return x + dot(h.astype(_BF16), w2_v[...])

    def q_all(x, q_ref):
        xn = layernorm(x).astype(_BF16)
        res = dot(xn, wq_v[...])
        for g in range(HKV):
            q_ref[g] = (pick_heads(res[:, g * G:(g + 1) * G]) * qscale).astype(_BF16)

    def wo_all(lo):
        lhs = jnp.concatenate([block_diag(o_v[g]) for g in range(HKV)], axis=1)
        return sum_rows(dot(lhs, wo_v[...]), lo, REP)

    c_x().wait()
    c_wq().wait()
    c_k1a().start()
    xin = x_v[...].astype(_F32)
    x0 = jnp.broadcast_to(xin[0:1, :], (_ROWS, D))
    x1 = jnp.broadcast_to(xin[1:2, :], (_ROWS, D))
    x01 = jnp.where(row_d < REP, x0, x1)
    q_all(x01, q1_v)

    ones = jnp.ones((_ROWS, D), _BF16)
    csq = dot(ones, wq_v[...])
    for g in range(HKV):
        csq_v[g] = pick_heads(csq[:, g * G:(g + 1) * G])
    c_wo().wait()
    c_w1().wait()
    c_w2().wait()
    c_k1b().start()
    cs1_v[...] = dot(ones, w1_v[...])
    for src, dst in ((wq_v, wqp_v), (wo_v, wop_v), (w1_v, w1p_v), (w2_v, w2p_v)):
        def pack_rows(i, carry, src=src, dst=dst):
            r0 = pl.multiple_of(i * 64, 64)
            r1 = pl.multiple_of(i * 32, 32)
            dst[pl.ds(r1, 32), :] = pack(src[pl.ds(r0, 64), :])
            return carry
        lax.fori_loop(0, src.shape[0] // 64, pack_rows, 0)
    w1t = w1_v[:, FM:F].astype(_F32).T
    w1t_v[...] = w1t
    w2f_v[...] = w2_v[FM:F, :].astype(_F32)
    w1s = jnp.broadcast_to(jnp.sum(w1t, axis=1, keepdims=True), (_FV, DH))
    ccat = jnp.zeros((_ROWS, DH), _F32)
    for nb in range(_NBT):
        ccat = jnp.where(lane == nb, w1s[nb * 8:(nb + 1) * 8, :], ccat)
    cs1c_v[0:_FV, :] = w1s
    cs1c_v[_FV:_FV + 8, :] = ccat
    for c in col_v:
        c[2 * DH:2 * DH + 8, :] = jnp.zeros((8, DH), _U32)

    c_k0().wait()
    c_v1a().start()

    def qk0_head(h, carry):
        s = lax.dot_general(q1_v[h], k_v[0, h], _NT, preferred_element_type=_F32)
        p, _, l = softmax_p(s)
        p_v[h] = p
        linv_v[h] = jnp.broadcast_to(1.0 / l, (_ROWS, DH))
        return carry
    lax.fori_loop(0, HKV, qk0_head, 0)

    def pv0_head(h, carry):
        @pl.when(h == 0)
        def _():
            c_v0a().wait()
            c_v1b().start()

        @pl.when(h == HH)
        def _():
            c_v0b().wait()
            c_vt(0).start()
        o_v[h] = dot(p_v[h], v_v[0, h]) * linv_v[h]
        return carry
    lax.fori_loop(0, HKV, pv0_head, 0)

    x0 = x0 + wo_all(0)
    x0 = ffn(x0)
    q_all(x0, q2_v)

    def attn0_head(h, carry):
        s = lax.dot_general(q2_v[h], k_v[0, h], _NT, preferred_element_type=_F32)
        p, _, l = softmax_p(s)
        o_v[h] = dot(p, v_v[0, h]) * (1.0 / l)
        return carry
    lax.fori_loop(0, HKV, attn0_head, 0)
    x0 = x0 + wo_all(0)
    x0 = ffn(x0)

    eye = (lax.broadcasted_iota(jnp.int32, (DH, DH), 0)
           == lax.broadcasted_iota(jnp.int32, (DH, DH), 1)).astype(_BF16)

    def qkt_head(h, carry):
        @pl.when(h == 0)
        def _():
            c_k1a().wait()
            c_vt(1).start()

        @pl.when(h == HH)
        def _():
            c_k1b().wait()
            c_vt(2).start()
        q = q1_v[h]
        lhs = jnp.concatenate([eye, q, q], axis=0)
        r = lax.dot_general(lhs, k_v[1, h], _NT, preferred_element_type=_F32)
        kt_v[h, 0:DH // 2, :] = pack(r[:DH, :HALF].astype(_BF16))
        kt_v[h, DH // 2:DH, :] = pack(r[:DH, HALF:].astype(_BF16))
        p, _, l = softmax_p(r[DH:DH + _ROWS])
        p_v[h] = p
        linv_v[h] = jnp.broadcast_to(1.0 / l, (_ROWS, DH))
        return carry + h
    zero = lax.fori_loop(0, HKV, qkt_head, 0) - (HKV * (HKV - 1)) // 2
    zero = jnp.clip(zero, 0, 1)

    def pv1_head(h, acc):
        @pl.when(h == 0)
        def _():
            c_v1a().wait()

        @pl.when(h == _V1_SPLIT)
        def _():
            c_v1b().wait()
        o = dot(p_v[h], v_v[1, h]) * linv_v[h]
        w = wo_v[pl.ds(pl.multiple_of(h * G, G), G), :]
        return acc + dot(block_diag(o), w)
    acc = lax.fori_loop(0, HL, pv1_head, jnp.zeros((_ROWS, D), _F32))

    _, x1c, _ = ln_stats(x1)
    upd = sum_rows(acc, REP, REP)
    y_part = x1c + upd
    x_part = x1 + upd

    def ffn_tail(x, y):
        yb = y.astype(_BF16)
        yf = yb.astype(_F32)
        m, yc, r = ln_stats1(yf)
        rh = 0.5 * r
        hh = (dot(yb, unpack(w1p_v[:, 0:FM])) - m * cs1_v[:, 0:FM]) * rh
        upd = dot(silu_half(hh).astype(_BF16), unpack(w2p_v[0:FM // 2, :]))
        nblk = _FV // 8
        hs = []
        for nb in range(nblk):
            t = w1t_v[nb * 8:(nb + 1) * 8, :] * yf
            t = (t[:, 0:DH] + t[:, DH:2 * DH]) + (t[:, 2 * DH:3 * DH] + t[:, 3 * DH:])
            hs.append(jnp.broadcast_to(jnp.sum(t, axis=1, keepdims=True), (_ROWS, DH)))
        hcat = hs[0]
        for nb in range(1, _NBT):
            hcat = jnp.where(lane == nb, hs[nb], hcat)
        hcat = silu_half((hcat - m * cs1c_v[_FV:_FV + 8, :]) * rh)
        a = None
        for nb in list(range(_NBT, nblk)) + list(range(_NBT)):
            if nb < _NBT:
                hc = jnp.broadcast_to(hcat[:, nb:nb + 1], (_ROWS, DH))
            else:
                hc = silu_half((hs[nb] - m * cs1c_v[nb * 8:(nb + 1) * 8, :]) * rh)
            u = w2f_v[nb * 8:(nb + 1) * 8, :] * jnp.concatenate([hc] * (D // DH), axis=1)
            a = u if a is None else a + u
        upd = upd + sum_rows(a, 0, _ROWS)
        return x + upd, yc + upd

    for i, (o_, n) in enumerate(tail_offs):
        c_vt(i).wait()
        o = dot(p_v[HL, :, o_:o_ + n], v_v[1, HL, o_:o_ + n, :])
        if i > 0:
            o = o + o_v[HL]
        if i + 1 < len(tail_offs):
            o_v[HL] = o
    o = o * linv_v[HL]
    upd = sum_rows(dot(block_diag(o), unpack(wop_v[HL * G // 2:(HL + 1) * G // 2, :])),
                   REP, REP)
    x1, y = ffn_tail(x_part + upd, y_part + upd)

    def to_col(rows, col_ref):
        u = [pltpu.bitcast(jnp.broadcast_to(r_, (_ROWS, DH)), _U32) for r_ in rows]
        pk = [(u[0] >> 16) | u[1], (u[2] >> 16) | u[3]]
        rep = jnp.concatenate(
            [jnp.broadcast_to(p_[0:1, :], (DH, DH)) for p_ in pk], axis=1)
        col_ref[0:2 * DH, :] = rep.T

    def col_pair(col_ref, i):
        u = col_ref[pl.ds(pl.multiple_of((zero + i) * 8, 8), 8), :]
        return (pltpu.bitcast(u << 16, _F32),
                pltpu.bitcast(u & jnp.uint32(0xFFFF0000), _F32))

    toks = []

    def gate(x):
        while toks:
            x = jnp.where(zero != 0, toks.pop().astype(x.dtype), x)
        return x

    last = [None] * 4

    def vpu_matvec(col_ref, wp_ref, r0, c0):
        accs = [None] * 4
        for p_ in range(2):
            for kb in range(DH // 16):
                cks = [col_pair(col_ref, p_ * (DH // 8) + kb * 2 + sub)
                       for sub in range(2)]
                for hl in range(2):
                    rr = (r0 + (2 * p_ + hl) * DH) // 2 + kb * 8
                    ws = [unpack(wp_ref[rr:rr + 8, c0 + j * DH:c0 + (j + 1) * DH]
                                 ).astype(_F32) for j in range(4)]
                    for sub in range(2):
                        for j in range(4):
                            t = ws[j][sub * 8:(sub + 1) * 8, :] * cks[sub][hl]
                            accs[j] = t if accs[j] is None else accs[j] + t
        last[:] = accs
        return accs

    def fold_rows(a):
        def fold(x, y_, sh):
            msk = (row % (2 * sh)) < sh
            if 2 * sh == _ROWS:
                return (jnp.where(msk, x, y_)
                        + pltpu.roll(jnp.where(msk, y_, x), sh, axis=0))
            return jnp.where(msk, x + pltpu.roll(x, _ROWS - sh, axis=0),
                             y_ + pltpu.roll(y_, sh, axis=0))
        b = [fold(a[i], a[i + 4], 4) for i in range(4)]
        c = [fold(b[i], b[i + 2], 2) for i in range(2)]
        return fold(c[0], c[1], 1)

    yb = y.astype(_BF16)
    yf = yb.astype(_F32)
    m, yc, r = ln_stats1(yf)
    rq = r * qscale
    to_col([yf[0:1, j * DH:(j + 1) * DH] for j in range(D // DH)], col_v[0])
    qb, sm, ps, oh, os_ = {}, {}, {}, {}, {}
    st = {"mx": None, "vp": None}

    def finish_q(g, res):
        qb[g] = ((res - m * csq_v[g]) * rq).astype(_BF16)

    def t_mq(g):
        finish_q(g, pick_heads(dot(yb, unpack(wqp_v[:, g * G:(g + 1) * G]))))

    def t_wq(g):
        accs = vpu_matvec(col_v[0], wqp_v, 0, g * G)
        finish_q(g, fold_rows(accs + accs))

    def t_tk():
        toks.append((last[0] + last[1]) + (last[2] + last[3]))

    def t_q(g, part):
        q = gate(qb[g])
        zq = jnp.zeros_like(q)
        q2 = jnp.concatenate(
            [jnp.where(lo_rows, q, zq), jnp.where(lo_rows, zq, q)], axis=1)
        c0 = part * (HALF // 2)
        sm.setdefault(g, []).append(dot(q2, unpack(kt_v[g, :, c0:c0 + HALF // 2])))

    def t_sm(g):
        p, mx, l = softmax_p(jnp.concatenate(sm.pop(g), axis=1))
        mx = jnp.broadcast_to(mx, (_ROWS, DH))
        l = jnp.broadcast_to(l, (_ROWS, DH))
        mx_all = jnp.maximum(mx, pltpu.roll(mx, REP, axis=0))
        a = jnp.exp2(mx - mx_all)
        al = a * l
        ps[g] = (p, a / (al + pltpu.roll(al, REP, axis=0)))

    def t_p(g, part):
        if g not in ps:
            t_sm(g)
        p, c = ps[g]
        if toks:
            tk = list(toks)
            pieces = []
            for i in range(4):
                toks[:] = tk
                pieces.append(gate(p[:, i * DH:(i + 1) * DH]))
            p = jnp.concatenate(pieces + [p[:, 4 * DH:]], axis=1)
        o = dot(p, v_v[1, g, part * HALF:(part + 1) * HALF, :])
        if part == 0:
            oh[g] = o
        else:
            os_[g] = jnp.where(lo_rows, oh.pop(g), o) * c

    def t_mo(g):
        part = dot(block_diag(gate(os_.pop(g))),
                   unpack(wop_v[g * G // 2:(g + 1) * G // 2, :]))
        st["mx"] = part if st["mx"] is None else part + st["mx"]

    def t_wo(g):
        o = os_.pop(g)
        o4 = (o + pltpu.roll(o, REP, axis=0)).astype(_BF16).astype(_F32)
        to_col([o4[j:j + 1, :] for j in range(REP)], col_v[1 + g])
        part = jnp.concatenate(vpu_matvec(col_v[1 + g], wop_v, g * G, 0), axis=1)
        st["vp"] = part if st["vp"] is None else st["vp"] + part

    tasks = {"mq": t_mq, "wq": t_wq, "tk": t_tk, "mo": t_mo, "wo": t_wo,
             "qa": lambda g: t_q(g, 0), "qb": lambda g: t_q(g, 1),
             "pl": lambda g: t_p(g, 0), "ph": lambda g: t_p(g, 1)}
    for item in _SCHED.split():
        tasks[item[:2]](*[int(c) for c in item[2:]])
    assert not os_ and not toks
    upd = sum_rows(st["mx"] + st["vp"], 0, _ROWS)
    x1, _ = ffn_tail(x1 + upd, yc + upd)
    out = jnp.where(row_d < 1, x0, x1)
    o_ref[...] = out[0:B, :].astype(o_ref.dtype)


@jax.jit
def pallas_interleave_layers__gqa_block_cached__dense_activation_silu__decode_kernel(
    A_x: jax.Array,
    A_k_cache: jax.Array,
    A_v_cache: jax.Array,
    A_wq: jax.Array,
    A_wo: jax.Array,
    B_x: jax.Array,
    B_w1: jax.Array,
    B_w2: jax.Array,
):
    del B_x
    B, SQ, D = A_x.shape
    _, HKV, SK, DH = A_k_cache.shape
    HQ = A_wq.shape[1] // DH
    REP = HQ // HKV
    F = B_w1.shape[1]
    assert B == 2 and SQ == 1 and 2 * REP == _ROWS and HKV == 8
    assert D == REP * DH and DH == 128
    dims = (B, D, HKV, SK, DH, REP, F)

    def kernel(*refs):
        _kernel_body(dims, *refs)

    any_spec = pl.BlockSpec(memory_space=pl.ANY)
    out = pl.pallas_call(
        kernel,
        out_shape=jax.ShapeDtypeStruct((B, D), A_x.dtype),
        in_specs=[any_spec] * 7,
        out_specs=pl.BlockSpec(memory_space=pltpu.VMEM),
        scratch_shapes=[
            pltpu.VMEM((B, D), _BF16),
            pltpu.VMEM((B, HKV, SK, DH), _BF16),
            pltpu.VMEM((B, HKV, SK, DH), _BF16),
            pltpu.VMEM((HKV, DH, SK // 2), _U32),
            pltpu.VMEM((D, HQ * DH), _BF16),
            pltpu.VMEM((HQ * DH, D), _BF16),
            pltpu.VMEM((D, F), _BF16),
            pltpu.VMEM((F, D), _BF16),
            pltpu.VMEM((HKV, _ROWS, DH), _BF16),
            pltpu.VMEM((HKV, _ROWS, DH), _BF16),
            pltpu.VMEM((HKV, _ROWS, SK), _BF16),
            pltpu.VMEM((HKV, _ROWS, DH), _F32),
            pltpu.VMEM((HKV, _ROWS, DH), _F32),
            pltpu.VMEM((HKV, _ROWS, DH), _F32),
            pltpu.VMEM((_ROWS, F), _F32),
            pltpu.VMEM((D // 2, HQ * DH), _U32),
            pltpu.VMEM((HQ * DH // 2, D), _U32),
            pltpu.VMEM((D // 2, F), _U32),
            pltpu.VMEM((F // 2, D), _U32),
            pltpu.VMEM((_FV, D), _F32),
            pltpu.VMEM((_FV + 8, DH), _F32),
            pltpu.VMEM((_FV, D), _F32),
            *[pltpu.VMEM((2 * DH + 8, DH), _U32) for _ in range(_N_COLS)],
            pltpu.SemaphoreType.DMA((_N_SEMS,)),
        ],
        compiler_params=pltpu.CompilerParams(
            vmem_limit_bytes=118 * 1024 * 1024),
    )(A_x.reshape(B, D), A_k_cache, A_v_cache, A_wq, A_wo, B_w1, B_w2)
    return out.reshape(B, SQ, D)
```

```python
import jax
import jax.numpy as jnp
from jax import lax
import jax.experimental.pallas as pl
import jax.experimental.pallas.tpu as pltpu

_BF16 = jnp.bfloat16
_F32 = jnp.float32
_U32 = jnp.uint32
_NT = (((1,), (1,)), ((), ()))
_LN_EPS = 1e-5
_ROWS = 8
_LOG2E = 1.4426950408889634

_TAIL_SPLITS = (6144, 1536, 512)
_N_SEMS = 5
_V1_SPLIT = 5
_FV = 768
_NBT = 40
_N_COLS = 7

_SCHED = ("mq0 wq1 wq2 wq3 wq4 wq5 wq6 wq7 qa0 qb0 qa1 qb1 pl0 ph0 qa2 qb2 "
          "pl1 ph1 qa3 wo0 tk qb3 pl2 ph2 qa4 wo1 tk qb4 pl3 ph3 qa5 wo2 tk "
          "qb5 pl4 ph4 qa6 wo3 tk qb6 pl5 ph5 qa7 wo4 tk qb7 pl6 ph6 pl7 "
          "wo5 tk ph7 mo6 mo7")


def _kernel_body(dims, x_hbm, k_hbm, v_hbm, wq_hbm, wo_hbm, w1_hbm, w2_hbm,
                 o_ref,
                 x_v, k_v, v_v, kt_v, wq_v, wo_v, w1_v, w2_v,
                 q1_v, q2_v, p_v, linv_v, o_v, csq_v, cs1_v,
                 wqp_v, wop_v, w1p_v, w2p_v, w1t_v, cs1c_v, w2f_v,
                 *rest):
    col_v, sems = rest[:_N_COLS], rest[_N_COLS]
    B, D, HKV, SK, DH, REP, F = dims
    G = REP * DH
    HALF = SK // 2
    HH = HKV // 2
    HL = HKV - 1
    FM = F - _FV
    qscale = (DH ** -0.5) * _LOG2E

    def cp(src, dst, i):
        return pltpu.make_async_copy(src, dst, sems.at[i])

    def kv_cp(hbm, vm, b, h0, h1, i):
        return cp(hbm.at[b, pl.ds(h0, h1 - h0)], vm.at[b, pl.ds(h0, h1 - h0)], i)

    tail_offs = []
    off = 0
    for n in _TAIL_SPLITS:
        tail_offs.append((off, n))
        off += n
    assert off == SK and len(tail_offs) == 3

    c_x = lambda: cp(x_hbm, x_v, 0)
    c_wq = lambda: cp(wq_hbm, wq_v, 0)
    c_wo = lambda: cp(wo_hbm, wo_v, 1)
    c_w1 = lambda: cp(w1_hbm, w1_v, 1)
    c_w2 = lambda: cp(w2_hbm, w2_v, 1)
    c_k0 = lambda: kv_cp(k_hbm, k_v, 0, 0, HKV, 2)
    c_v0a = lambda: kv_cp(v_hbm, v_v, 0, 0, HH, 3)
    c_v0b = lambda: kv_cp(v_hbm, v_v, 0, HH, HKV, 4)
    c_k1a = lambda: kv_cp(k_hbm, k_v, 1, 0, HH, 0)
    c_k1b = lambda: kv_cp(k_hbm, k_v, 1, HH, HKV, 1)
    c_v1a = lambda: kv_cp(v_hbm, v_v, 1, 0, _V1_SPLIT, 2)
    c_v1b = lambda: kv_cp(v_hbm, v_v, 1, _V1_SPLIT, HL, 3)

    def c_vt(i):
        o, n = tail_offs[i]
        return cp(v_hbm.at[1, HL, pl.ds(o, n)], v_v.at[1, HL, pl.ds(o, n)],
                  (4, 0, 1)[i])

    for c in (c_wq, c_x, c_wo, c_w1, c_w2, c_k0, c_v0a, c_v0b):
        c().start()

    row = lax.broadcasted_iota(jnp.int32, (_ROWS, DH), 0)
    lane = lax.broadcasted_iota(jnp.int32, (_ROWS, DH), 1)
    row_in_grp = row % REP
    lo_rows = row < REP
    row_d = lax.broadcasted_iota(jnp.int32, (_ROWS, D), 0)

    def dot(a, b):
        return jnp.dot(a, b, preferred_element_type=_F32)

    def pack(x):
        return pltpu.bitcast(x, _U32)

    def unpack(x):
        return pltpu.bitcast(x, _BF16)

    def ln_stats(x):
        m = jnp.mean(x, axis=-1, keepdims=True)
        xc = x - m
        var = jnp.mean(xc * xc, axis=-1, keepdims=True)
        return m, xc, lax.rsqrt(var + _LN_EPS)

    def ln_stats1(x):
        m = jnp.mean(x, axis=-1, keepdims=True)
        m2 = jnp.mean(x * x, axis=-1, keepdims=True)
        var = jnp.maximum(m2 - m * m, 0.0)
        return m, lax.rsqrt(var + _LN_EPS)

    def layernorm(x):
        _, xc, r = ln_stats(x)
        return xc * r

    def pick_heads(res):
        q = res[:, 0:DH]
        for j in range(1, REP):
            q = jnp.where(row_in_grp == j, res[:, j * DH:(j + 1) * DH], q)
        return q

    def softmax_p(s):
        m = jnp.max(s, axis=-1, keepdims=True)
        p = jnp.exp2(s - m)
        l = jnp.sum(p, axis=-1, keepdims=True)
        return p.astype(_BF16), m, l

    def block_diag(o):
        parts = [jnp.where(row_in_grp == j, o, 0.0) for j in range(REP)]
        return jnp.concatenate(parts, axis=1).astype(_BF16)

    def sum_rows(acc, lo, n):
        if n < _ROWS:
            valid = jnp.logical_and(row_d >= lo, row_d < lo + n)
            acc = jnp.where(valid, acc, 0.0)
        r = jnp.sum(acc, axis=0, keepdims=True)
        return jnp.broadcast_to(r, (_ROWS, D))

    def silu_half(hh):
        return hh + hh * jnp.tanh(hh)

    def ffn(x):
        xn = layernorm(x).astype(_BF16)
        h = silu_half(0.5 * dot(xn, w1_v[...]))
        return x + dot(h.astype(_BF16), w2_v[...])

    def q_all(x, q_ref):
        xn = layernorm(x).astype(_BF16)
        res = dot(xn, wq_v[...])
        for g in range(HKV):
            q_ref[g] = (pick_heads(res[:, g * G:(g + 1) * G]) * qscale).astype(_BF16)

    def wo_all(lo):
        lhs = jnp.concatenate([block_diag(o_v[g]) for g in range(HKV)], axis=1)
        return sum_rows(dot(lhs, wo_v[...]), lo, REP)

    c_x().wait()
    c_wq().wait()
    c_k1a().start()
    xin = x_v[...].astype(_F32)
    x0 = jnp.broadcast_to(xin[0:1, :], (_ROWS, D))
    x1 = jnp.broadcast_to(xin[1:2, :], (_ROWS, D))
    x01 = jnp.where(row_d < REP, x0, x1)
    q_all(x01, q1_v)

    ones = jnp.ones((_ROWS, D), _BF16)
    csq = dot(ones, wq_v[...])
    for g in range(HKV):
        csq_v[g] = pick_heads(csq[:, g * G:(g + 1) * G])
    c_wo().wait()
    c_w1().wait()
    c_w2().wait()
    c_k1b().start()
    cs1_v[...] = dot(ones, w1_v[...])
    for src, dst in ((wq_v, wqp_v), (wo_v, wop_v), (w1_v, w1p_v), (w2_v, w2p_v)):
        def pack_rows(i, carry, src=src, dst=dst):
            r0 = pl.multiple_of(i * 64, 64)
            r1 = pl.multiple_of(i * 32, 32)
            dst[pl.ds(r1, 32), :] = pack(src[pl.ds(r0, 64), :])
            return carry
        lax.fori_loop(0, src.shape[0] // 64, pack_rows, 0)
    w1t = w1_v[:, FM:F].astype(_F32).T
    w1t_v[...] = w1t
    w2f_v[...] = w2_v[FM:F, :].astype(_F32)
    w1s = jnp.broadcast_to(jnp.sum(w1t, axis=1, keepdims=True), (_FV, DH))
    ccat = jnp.zeros((_ROWS, DH), _F32)
    for nb in range(_NBT):
        ccat = jnp.where(lane == nb, w1s[nb * 8:(nb + 1) * 8, :], ccat)
    cs1c_v[0:_FV, :] = w1s
    cs1c_v[_FV:_FV + 8, :] = ccat
    for c in col_v:
        c[2 * DH:2 * DH + 8, :] = jnp.zeros((8, DH), _U32)

    c_k0().wait()
    c_v1a().start()

    def qk0_head(h, carry):
        s = lax.dot_general(q1_v[h], k_v[0, h], _NT, preferred_element_type=_F32)
        p, _, l = softmax_p(s)
        p_v[h] = p
        linv_v[h] = jnp.broadcast_to(1.0 / l, (_ROWS, DH))
        return carry
    lax.fori_loop(0, HKV, qk0_head, 0)

    def pv0_head(h, carry):
        @pl.when(h == 0)
        def _():
            c_v0a().wait()
            c_v1b().start()

        @pl.when(h == HH)
        def _():
            c_v0b().wait()
            c_vt(0).start()
        o_v[h] = dot(p_v[h], v_v[0, h]) * linv_v[h]
        return carry
    lax.fori_loop(0, HKV, pv0_head, 0)

    x0 = x0 + wo_all(0)
    x0 = ffn(x0)
    q_all(x0, q2_v)

    def attn0_head(h, carry):
        s = lax.dot_general(q2_v[h], k_v[0, h], _NT, preferred_element_type=_F32)
        p, _, l = softmax_p(s)
        o_v[h] = dot(p, v_v[0, h]) * (1.0 / l)
        return carry
    lax.fori_loop(0, HKV, attn0_head, 0)
    x0 = x0 + wo_all(0)
    x0 = ffn(x0)

    eye = (lax.broadcasted_iota(jnp.int32, (DH, DH), 0)
           == lax.broadcasted_iota(jnp.int32, (DH, DH), 1)).astype(_BF16)

    def qkt_head(h, carry):
        @pl.when(h == 0)
        def _():
            c_k1a().wait()
            c_vt(1).start()

        @pl.when(h == HH)
        def _():
            c_k1b().wait()
            c_vt(2).start()
        q = q1_v[h]
        lhs = jnp.concatenate([eye, q, q], axis=0)
        r = lax.dot_general(lhs, k_v[1, h], _NT, preferred_element_type=_F32)
        kt_v[h, 0:DH // 2, :] = pack(r[:DH, :HALF].astype(_BF16))
        kt_v[h, DH // 2:DH, :] = pack(r[:DH, HALF:].astype(_BF16))
        p, _, l = softmax_p(r[DH:DH + _ROWS])
        p_v[h] = p
        linv_v[h] = jnp.broadcast_to(1.0 / l, (_ROWS, DH))
        return carry + h
    zero = lax.fori_loop(0, HKV, qkt_head, 0) - (HKV * (HKV - 1)) // 2
    zero = jnp.clip(zero, 0, 1)

    def pv1_head(h, acc):
        @pl.when(h == 0)
        def _():
            c_v1a().wait()

        @pl.when(h == _V1_SPLIT)
        def _():
            c_v1b().wait()
        o = dot(p_v[h], v_v[1, h]) * linv_v[h]
        w = wo_v[pl.ds(pl.multiple_of(h * G, G), G), :]
        return acc + dot(block_diag(o), w)
    acc = lax.fori_loop(0, HL, pv1_head, jnp.zeros((_ROWS, D), _F32))

    x_part = x1 + sum_rows(acc, REP, REP)
    y_part = x_part - jnp.mean(x_part, axis=-1, keepdims=True)

    def ffn_tail(x, y):
        yb = y.astype(_BF16)
        yf = yb.astype(_F32)
        m, r = ln_stats1(yf)
        rh = 0.5 * r
        hh = (dot(yb, unpack(w1p_v[:, 0:FM])) - m * cs1_v[:, 0:FM]) * rh
        upd = dot(silu_half(hh).astype(_BF16), unpack(w2p_v[0:FM // 2, :]))
        nblk = _FV // 8
        hs = []
        for nb in range(nblk):
            t = w1t_v[nb * 8:(nb + 1) * 8, :] * yf
            t = (t[:, 0:DH] + t[:, DH:2 * DH]) + (t[:, 2 * DH:3 * DH] + t[:, 3 * DH:])
            hs.append(jnp.broadcast_to(jnp.sum(t, axis=1, keepdims=True), (_ROWS, DH)))
        hcat = hs[0]
        for nb in range(1, _NBT):
            hcat = jnp.where(lane == nb, hs[nb], hcat)
        hcat = silu_half((hcat - m * cs1c_v[_FV:_FV + 8, :]) * rh)
        a = None
        for nb in list(range(_NBT, nblk)) + list(range(_NBT)):
            if nb < _NBT:
                hc = jnp.broadcast_to(hcat[:, nb:nb + 1], (_ROWS, DH))
            else:
                hc = silu_half((hs[nb] - m * cs1c_v[nb * 8:(nb + 1) * 8, :]) * rh)
            u = w2f_v[nb * 8:(nb + 1) * 8, :] * jnp.concatenate([hc] * (D // DH), axis=1)
            a = u if a is None else a + u
        upd = upd + sum_rows(a, 0, _ROWS)
        return x + upd, (y - m) + upd

    for i, (o_, n) in enumerate(tail_offs):
        c_vt(i).wait()
        o = dot(p_v[HL, :, o_:o_ + n], v_v[1, HL, o_:o_ + n, :])
        if i > 0:
            o = o + o_v[HL]
        if i + 1 < len(tail_offs):
            o_v[HL] = o
    o = o * linv_v[HL]
    upd = sum_rows(dot(block_diag(o), unpack(wop_v[HL * G // 2:(HL + 1) * G // 2, :])),
                   REP, REP)
    x1, y = ffn_tail(x_part + upd, y_part + upd)

    def to_col(rows, col_ref):
        u = [pltpu.bitcast(jnp.broadcast_to(r_, (_ROWS, DH)), _U32) for r_ in rows]
        hi = jnp.uint32(0xFFFF0000)
        pk = [(u[0] >> 16) | (u[1] & hi), (u[2] >> 16) | (u[3] & hi)]
        rep = jnp.concatenate(
            [jnp.broadcast_to(p_[0:1, :], (DH, DH)) for p_ in pk], axis=1)
        col_ref[0:2 * DH, :] = rep.T

    def col_pair(col_ref, i):
        u = col_ref[pl.ds(pl.multiple_of((zero + i) * 8, 8), 8), :]
        return (pltpu.bitcast(u << 16, _F32),
                pltpu.bitcast(u & jnp.uint32(0xFFFF0000), _F32))

    toks = []

    def gate(x):
        while toks:
            x = jnp.where(zero != 0, toks.pop().astype(x.dtype), x)
        return x

    last = [None] * 4

    def vpu_matvec(col_ref, wp_ref, r0, c0):
        accs = [None] * 4
        for p_ in range(2):
            for kb in range(DH // 16):
                cks = [col_pair(col_ref, p_ * (DH // 8) + kb * 2 + sub)
                       for sub in range(2)]
                for hl in range(2):
                    rr = (r0 + (2 * p_ + hl) * DH) // 2 + kb * 8
                    ws = [unpack(wp_ref[rr:rr + 8, c0 + j * DH:c0 + (j + 1) * DH]
                                 ).astype(_F32) for j in range(4)]
                    for sub in range(2):
                        for j in range(4):
                            t = ws[j][sub * 8:(sub + 1) * 8, :] * cks[sub][hl]
                            accs[j] = t if accs[j] is None else accs[j] + t
        last[:] = accs
        return accs

    def fold_rows(a):
        def fold(x, y_, sh):
            msk = (row % (2 * sh)) < sh
            if 2 * sh == _ROWS:
                return (jnp.where(msk, x, y_)
                        + pltpu.roll(jnp.where(msk, y_, x), sh, axis=0))
            return jnp.where(msk, x + pltpu.roll(x, _ROWS - sh, axis=0),
                             y_ + pltpu.roll(y_, sh, axis=0))
        b = [fold(a[i], a[i + 4], 4) for i in range(4)]
        c = [fold(b[i], b[i + 2], 2) for i in range(2)]
        return fold(c[0], c[1], 1)

    yb = y.astype(_BF16)
    yf = yb.astype(_F32)
    m, r = ln_stats1(yf)
    yc = y - m
    rq = r * qscale
    to_col([yf[0:1, j * DH:(j + 1) * DH] for j in range(D // DH)], col_v[0])
    qb, sm, ps, oh, os_ = {}, {}, {}, {}, {}
    st = {"mx": None, "vp": None}

    def finish_q(g, res):
        qb[g] = ((res - m * csq_v[g]) * rq).astype(_BF16)

    def t_mq(g):
        finish_q(g, pick_heads(dot(yb, unpack(wqp_v[:, g * G:(g + 1) * G]))))

    def t_wq(g):
        accs = vpu_matvec(col_v[0], wqp_v, 0, g * G)
        finish_q(g, fold_rows(accs + accs))

    def t_tk():
        toks.append((last[0] + last[1]) + (last[2] + last[3]))

    def t_q(g, part):
        q = gate(qb[g])
        zq = jnp.zeros_like(q)
        q2 = jnp.concatenate(
            [jnp.where(lo_rows, q, zq), jnp.where(lo_rows, zq, q)], axis=1)
        c0 = part * (HALF // 2)
        sm.setdefault(g, []).append(dot(q2, unpack(kt_v[g, :, c0:c0 + HALF // 2])))

    def t_sm(g):
        p, mx, l = softmax_p(jnp.concatenate(sm.pop(g), axis=1))
        mx = jnp.broadcast_to(mx, (_ROWS, DH))
        l = jnp.broadcast_to(l, (_ROWS, DH))
        mx_all = jnp.maximum(mx, pltpu.roll(mx, REP, axis=0))
        a = jnp.exp2(mx - mx_all)
        al = a * l
        ps[g] = (p, a / (al + pltpu.roll(al, REP, axis=0)))

    def t_p(g, part):
        if g not in ps:
            t_sm(g)
        p, c = ps[g]
        if toks:
            tk = list(toks)
            pieces = []
            for i in range(4):
                toks[:] = tk
                pieces.append(gate(p[:, i * DH:(i + 1) * DH]))
            p = jnp.concatenate(pieces + [p[:, 4 * DH:]], axis=1)
        o = dot(p, v_v[1, g, part * HALF:(part + 1) * HALF, :])
        if part == 0:
            oh[g] = o
        else:
            os_[g] = jnp.where(lo_rows, oh.pop(g), o) * c

    def t_mo(g):
        part = dot(block_diag(gate(os_.pop(g))),
                   unpack(wop_v[g * G // 2:(g + 1) * G // 2, :]))
        st["mx"] = part if st["mx"] is None else part + st["mx"]

    def t_wo(g):
        o = os_.pop(g)
        o4 = (o + pltpu.roll(o, REP, axis=0)).astype(_BF16).astype(_F32)
        to_col([o4[j:j + 1, :] for j in range(REP)], col_v[1 + g])
        part = jnp.concatenate(vpu_matvec(col_v[1 + g], wop_v, g * G, 0), axis=1)
        st["vp"] = part if st["vp"] is None else st["vp"] + part

    tasks = {"mq": t_mq, "wq": t_wq, "tk": t_tk, "mo": t_mo, "wo": t_wo,
             "qa": lambda g: t_q(g, 0), "qb": lambda g: t_q(g, 1),
             "pl": lambda g: t_p(g, 0), "ph": lambda g: t_p(g, 1)}
    for item in _SCHED.split():
        tasks[item[:2]](*[int(c) for c in item[2:]])
    assert not os_ and not toks
    upd = sum_rows(st["mx"] + st["vp"], 0, _ROWS)
    x1, _ = ffn_tail(x1 + upd, yc + upd)
    out = jnp.where(row_d < 1, x0, x1)
    o_ref[...] = out[0:B, :].astype(o_ref.dtype)


@jax.jit
def pallas_interleave_layers__gqa_block_cached__dense_activation_silu__decode_kernel(
    A_x: jax.Array,
    A_k_cache: jax.Array,
    A_v_cache: jax.Array,
    A_wq: jax.Array,
    A_wo: jax.Array,
    B_x: jax.Array,
    B_w1: jax.Array,
    B_w2: jax.Array,
):
    del B_x
    B, SQ, D = A_x.shape
    _, HKV, SK, DH = A_k_cache.shape
    HQ = A_wq.shape[1] // DH
    REP = HQ // HKV
    F = B_w1.shape[1]
    assert B == 2 and SQ == 1 and 2 * REP == _ROWS and HKV == 8
    assert D == REP * DH and DH == 128
    dims = (B, D, HKV, SK, DH, REP, F)

    def kernel(*refs):
        _kernel_body(dims, *refs)

    any_spec = pl.BlockSpec(memory_space=pl.ANY)
    out = pl.pallas_call(
        kernel,
        out_shape=jax.ShapeDtypeStruct((B, D), A_x.dtype),
        in_specs=[any_spec] * 7,
        out_specs=pl.BlockSpec(memory_space=pltpu.VMEM),
        scratch_shapes=[
            pltpu.VMEM((B, D), _BF16),
            pltpu.VMEM((B, HKV, SK, DH), _BF16),
            pltpu.VMEM((B, HKV, SK, DH), _BF16),
            pltpu.VMEM((HKV, DH, SK // 2), _U32),
            pltpu.VMEM((D, HQ * DH), _BF16),
            pltpu.VMEM((HQ * DH, D), _BF16),
            pltpu.VMEM((D, F), _BF16),
            pltpu.VMEM((F, D), _BF16),
            pltpu.VMEM((HKV, _ROWS, DH), _BF16),
            pltpu.VMEM((HKV, _ROWS, DH), _BF16),
            pltpu.VMEM((HKV, _ROWS, SK), _BF16),
            pltpu.VMEM((HKV, _ROWS, DH), _F32),
            pltpu.VMEM((HKV, _ROWS, DH), _F32),
            pltpu.VMEM((HKV, _ROWS, DH), _F32),
            pltpu.VMEM((_ROWS, F), _F32),
            pltpu.VMEM((D // 2, HQ * DH), _U32),
            pltpu.VMEM((HQ * DH // 2, D), _U32),
            pltpu.VMEM((D // 2, F), _U32),
            pltpu.VMEM((F // 2, D), _U32),
            pltpu.VMEM((_FV, D), _F32),
            pltpu.VMEM((_FV + 8, DH), _F32),
            pltpu.VMEM((_FV, D), _F32),
            *[pltpu.VMEM((2 * DH + 8, DH), _U32) for _ in range(_N_COLS)],
            pltpu.SemaphoreType.DMA((_N_SEMS,)),
        ],
        compiler_params=pltpu.CompilerParams(
            vmem_limit_bytes=118 * 1024 * 1024),
    )(A_x.reshape(B, D), A_k_cache, A_v_cache, A_wq, A_wo, B_w1, B_w2)
    return out.reshape(B, SQ, D)
```
